```python
import os as _os
_os.environ.setdefault("JAX_PLATFORMS", "cpu")
import jax
import jax.numpy as jnp

def _softmax(x, axis=-1):
    return jax.nn.softmax(x, axis=axis)
def _gelu(x):
    return jax.nn.gelu(x, approximate=True)
def _silu(x):
    return jax.nn.silu(x)
def _sigmoid(x):
    return jax.nn.sigmoid(x)
def _layernorm(x, axis=-1, eps=1e-5):
    m = jnp.mean(x, axis=axis, keepdims=True)
    v = jnp.var(x, axis=axis, keepdims=True)
    return (x - m) / jnp.sqrt(v + eps)
def _scatter_add(tgt, idx, src, axis=0):
    return tgt.at[idx].add(src)
def _segment_sum(src, seg, n):
    return jax.ops.segment_sum(src, seg, n)
class _Rng:
    def __init__(self, key):
        self._k = key
    def _next(self):
        self._k, sub = jax.random.split(self._k)
        return sub
    def normal(self, shape):
        return jax.random.normal(self._next(), shape, dtype=jnp.bfloat16)
    def randint(self, lo, hi, shape):
        return jax.random.randint(self._next(), shape, lo, hi, dtype=jnp.int32)
    def uniform(self, shape, lo=0.0, hi=1.0):
        return jax.random.uniform(self._next(), shape, jnp.bfloat16, lo, hi)
    def permutation(self, n):
        return jax.random.permutation(self._next(), n)


kernel_name = 'sequential_preLN__softmax_full_mha__dense_activation_gelu__prompt'

def setup_inputs():
    _rng = _Rng(jax.random.key(int.from_bytes(__import__("os").urandom(4), "little")))
    _w = (lambda a: (lambda t: t.astype(jnp.bfloat16) if jnp.issubdtype(t.dtype, jnp.floating) else t)(jnp.asarray(a)))
    def _A_setup():
        B, S, D = 1, 2048, 512
        return {
            "x": _w((lambda *s: _rng.normal(s) * 0.05)(B, S, D)),
            "wqkv": _w((lambda *s: _rng.normal(s) * 0.05)(D, 3 * D)),
            "wo": _w((lambda *s: _rng.normal(s) * 0.05)(D, D)),
        }
    _A_in = _A_setup()

    def _B_setup():
        B, S, D, F = 1, 2048, 512, 1792
        return {
            "x": _w((lambda *s: _rng.normal(s) * 0.05)(B, S, D)),
            "w1": _w((lambda *s: _rng.normal(s) * 0.4)(D, F) * (D ** -0.5)),
            "b1": _w((lambda *s: _rng.normal(s) * 0.4)(F) * 0.01),
            "w2": _w((lambda *s: _rng.normal(s) * 0.4)(F, D) * (F ** -0.5)),
            "b2": _w((lambda *s: _rng.normal(s) * 0.05)(D) * 0.01),
        }
    _B_in = _B_setup()

    return {
        "A_x": _A_in["x"],
        "A_wqkv": _A_in["wqkv"],
        "A_wo": _A_in["wo"],
        "B_x": _B_in["x"],
        "B_w1": _B_in["w1"],
        "B_b1": _B_in["b1"],
        "B_w2": _B_in["w2"],
        "B_b2": _B_in["b2"],
    }

def reference(A_x, A_wqkv, A_wo, B_x, B_w1, B_b1, B_w2, B_b2):
    def _A_ref(x, wqkv, wo):
        B, S, D = x.shape
        H = 32; Dh = D // H
        qkv = (lambda x, *d: x.transpose(*d))((x @ wqkv).reshape(B, S, 3, H, Dh), 2, 0, 3, 1, 4)
        q, k, v = qkv[0], qkv[1], qkv[2]
        scale = Dh ** -0.5
        scores = jnp.einsum("bhqd,bhkd->bhqk", q, k) * scale
        p = _softmax(scores, axis=-1)
        o = jnp.einsum("bhqk,bhkd->bhqd", p, v)
        return (lambda x, *d: x.transpose(*d))(o, 0, 2, 1, 3).reshape(B, S, D) @ wo

    def _B_ref(x, w1, b1, w2, b2):
        h = jnp.einsum("bsd,df->bsf", x, w1) + b1
        h = _gelu(h)
        return jnp.einsum("bsf,fd->bsd", h, w2) + b2

    x = A_x
    h = x + _A_ref(_layernorm(x, axis=-1), A_wqkv, A_wo)
    h2 = h + _B_ref(_layernorm(h, axis=-1), B_w1, B_b1, B_w2, B_b2)
    return h2
```

```python
import functools
import math

import jax
import jax.numpy as jnp
from jax import lax
import jax.experimental.pallas as pl
import jax.experimental.pallas.tpu as pltpu

BF = jnp.bfloat16
F32 = jnp.float32
U32 = jnp.uint32

H = 32
LN_EPS = 1e-5
LOG2E = 1.4426950408889634

TM1 = 512
TM3 = 256
TQ = 512
CK = 256
LAG = 1

SAFE_B = 60.0
SAFE_V_HI = 2.0 ** 40
SAFE_V_LO = 2.0 ** -40


def _nt(a, b):
    return lax.dot_general(a, b, (((1,), (1,)), ((), ())), preferred_element_type=F32)


def _layernorm(x):
    m = jnp.mean(x, axis=-1, keepdims=True)
    xc = x - m
    v = jnp.mean(xc * xc, axis=-1, keepdims=True)
    return xc * lax.rsqrt(v + LN_EPS)


def _gelu(x):
    c = math.sqrt(2.0 / math.pi)
    return 0.5 * x * (1.0 + jnp.tanh(c * (x + 0.044715 * (x * x * x))))


def _kernel(x_hbm, wqkv_hbm, wo_hbm, w1_hbm, b1_hbm, w2_hbm, b2_hbm, out_hbm,
            x_s, wqkv_s, wo_s, w1_s, b1_s, w2_s, b2_s, wqvt_s,
            k_s, qt_s, vt_s, qm_s, ot_s, st_s, out_s, sems, osems,
            *, S, D, F):
    DH = D // H
    NG = D // 128
    HPG = 128 // DH
    NLT = S // 128
    n1 = S // TM1
    n3 = S // TM3
    qscale = (DH ** -0.5) * LOG2E

    def cp(src, dst, i):
        return pltpu.make_async_copy(src, dst, sems.at[i])

    c_wqkv = cp(wqkv_hbm, wqkv_s, 0)
    c_x = [cp(x_hbm.at[pl.ds(i * TM1, TM1)], x_s.at[pl.ds(i * TM1, TM1)], 1 + i) for i in range(n1)]
    rest = [(wo_hbm, wo_s), (w1_hbm, w1_s), (b1_hbm, b1_s), (w2_hbm, w2_s), (b2_hbm, b2_s)]
    c_rest = [cp(s_, d_, 1 + n1 + i) for i, (s_, d_) in enumerate(rest)]
    c_x[0].start()
    c_wqkv.start()
    for c in c_x[1:]:
        c.start()
    for c in c_rest:
        c.start()

    qm_s[...] = jnp.zeros(qm_s.shape, qm_s.dtype)

    c_wqkv.wait()
    ri = lax.broadcasted_iota(jnp.int32, (128, 128), 0)
    ci = lax.broadcasted_iota(jnp.int32, (128, 128), 1)
    eye = jnp.where(ri == ci, 1.0, 0.0).astype(BF)
    for part, c0 in enumerate((0, 2 * D)):
        for b in range(NG):
            blk = _nt(eye, wqkv_s[:, c0 + b * 128:c0 + (b + 1) * 128])
            wqvt_s[part * D + b * 128:part * D + (b + 1) * 128, :] = blk.astype(BF)

    hi = lax.broadcasted_iota(jnp.int32, (H, D), 0)
    cj = lax.broadcasted_iota(jnp.int32, (H, D), 1)
    ind = jnp.where(cj // DH == hi, 1.0, 0.0).astype(BF)

    qmax = None
    kmax = None
    vmax = None
    for i in range(n1):
        c_x[i].wait()
        r0 = i * TM1
        xn = _layernorm(x_s[r0:r0 + TM1, :].astype(F32)).astype(BF)
        k = jnp.dot(xn, wqkv_s[:, D:2 * D], preferred_element_type=F32)
        kb = k.astype(BF)
        for g in range(NG):
            k_s[g, r0:r0 + TM1, :] = kb[:, g * 128:(g + 1) * 128]
        kf = kb.astype(F32)
        kn = _nt(ind, (kf * kf).astype(BF))
        kmax = kn if kmax is None else jnp.maximum(kmax, kn)
        qv = _nt(wqvt_s[...], xn)
        qb = (qv[:D] * qscale).astype(BF)
        vb = qv[D:].astype(BF)
        for t in range(TM1 // 128):
            lt = r0 // 128 + t
            qt_s[lt] = qb[:, t * 128:(t + 1) * 128]
            vt_s[lt] = vb[:, t * 128:(t + 1) * 128]
        qf = qb.astype(F32)
        qn = jnp.dot(ind, (qf * qf).astype(BF), preferred_element_type=F32)
        qmax = qn if qmax is None else jnp.maximum(qmax, qn)
        va = jnp.abs(vb.astype(F32)).reshape(D // 8, 8, TM1).max(axis=0)
        vmax = va if vmax is None else jnp.maximum(vmax, va)

    qh = jnp.max(qmax, axis=1, keepdims=True)
    kh = jnp.max(kmax, axis=1, keepdims=True)
    b2max = jnp.max(qh * kh) * 1.05
    vm = jnp.max(vmax)
    safe = jnp.logical_and(b2max <= SAFE_B * SAFE_B,
                           jnp.logical_and(vm <= SAFE_V_HI, vm >= SAFE_V_LO))

    nq = S // TQ
    nc = S // CK
    nlt = TQ // 128

    def prep_qm(h, hprev2, slot):
        jp = pl.multiple_of((hprev2 % HPG) * DH, DH)
        jn = pl.multiple_of((h % HPG) * DH, DH)
        rq = pl.multiple_of(h * DH, DH)
        qm_s[slot, :, pl.ds(jp, DH), :] = jnp.zeros((NLT, DH, 128), BF)
        qm_s[slot, :, pl.ds(jn, DH), :] = qt_s[:, pl.ds(rq, DH), :]

    def fast_head(h, carry):
        slot = h % 2
        g = h // HPG
        ro = pl.multiple_of(h * DH, DH)
        hn = jnp.minimum(h + 1, H - 1)
        T = nq * nc
        accs = {}
        ls = {}
        pv = {}

        def qk_part(t):
            qb_, c = divmod(t, nc)
            kc = k_s[g, c * CK:(c + 1) * CK, :]
            qm = jnp.concatenate([qm_s[slot, qb_ * nlt + b] for b in range(nlt)], axis=1)
            s = jnp.dot(kc, qm, preferred_element_type=F32)
            p = jnp.exp2(s)
            lp = p.reshape(CK // 8, 8, TQ).sum(axis=0)
            ls[qb_] = lp if qb_ not in ls else ls[qb_] + lp
            pv[t] = [p[kk * 128:(kk + 1) * 128].astype(BF) for kk in range(CK // 128)]

        def pv_part(t):
            qb_, c = divmod(t, nc)
            pbs = pv.pop(t)
            for kk in range(CK // 128):
                vt = vt_s[c * (CK // 128) + kk, pl.ds(ro, DH), :]
                dd = jnp.dot(vt, pbs[kk], preferred_element_type=F32)
                accs[qb_] = dd if qb_ not in accs else accs[qb_] + dd
            if c == nc - 1:
                lsum = jnp.sum(ls[qb_], axis=0, keepdims=True)
                ot_s[pl.ds(ro, DH), qb_ * TQ:(qb_ + 1) * TQ] = accs[qb_] / lsum

        for t in range(T + LAG):
            if t < T:
                qk_part(t)
            if t == 1:
                prep_qm(hn, jnp.maximum(h - 1, 0), 1 - slot)
            if t >= LAG:
                pv_part(t - LAG)
        return carry

    def slow_head(h, carry):
        slot = h % 2
        g = h // HPG
        ro = pl.multiple_of(h * DH, DH)
        hn = jnp.minimum(h + 1, H - 1)
        prep_qm(hn, jnp.maximum(h - 1, 0), 1 - slot)

        def qblock(qi, c2):
            qm = qm_s[slot, qi]
            st_s[...] = jnp.dot(k_s[g], qm, preferred_element_type=F32)
            m = jnp.max(st_s[...], axis=0, keepdims=True)
            acc = jnp.zeros((DH, 128), F32)
            l = jnp.zeros((1, 128), F32)
            for kt in range(NLT):
                p = jnp.exp2(st_s[kt * 128:(kt + 1) * 128, :] - m)
                l = l + jnp.sum(p, axis=0, keepdims=True)
                vt = vt_s[kt, pl.ds(ro, DH), :]
                acc = acc + jnp.dot(vt, p.astype(BF), preferred_element_type=F32)
            q0 = pl.multiple_of(qi * 128, 128)
            ot_s[pl.ds(ro, DH), pl.ds(q0, 128)] = acc / l
            return c2

        lax.fori_loop(0, NLT, qblock, 0)
        return carry

    prep_qm(0, 0, 0)

    @pl.when(safe)
    def _():
        lax.fori_loop(0, H, fast_head, 0)

    @pl.when(jnp.logical_not(safe))
    def _():
        lax.fori_loop(0, H, slow_head, 0)

    for c in c_rest:
        c.wait()

    def ocp(i, slot):
        return pltpu.make_async_copy(out_s.at[slot], out_hbm.at[pl.ds(i * TM3, TM3)], osems.at[slot])

    for i in range(n3):
        r0 = i * TM3
        slot = i % 2
        o = ot_s[:, r0:r0 + TM3].T.astype(BF)
        attn = jnp.dot(o, wo_s[...], preferred_element_type=F32)
        h = x_s[r0:r0 + TM3, :].astype(F32) + attn
        hn_ = _layernorm(h).astype(BF)
        u = jnp.dot(hn_, w1_s[...], preferred_element_type=F32) + b1_s[...].astype(F32)
        u = _gelu(u).astype(BF)
        y = jnp.dot(u, w2_s[...], preferred_element_type=F32) + b2_s[...].astype(F32)
        if i >= 2:
            ocp(i - 2, slot).wait()
        out_s[slot] = (h + y).astype(out_s.dtype)
        ocp(i, slot).start()
    for i in range(max(n3 - 2, 0), n3):
        ocp(i, i % 2).wait()


@jax.jit
def pallas_sequential_preLN__softmax_full_mha__dense_activation_gelu__prompt_kernel(
    A_x: jax.Array,
    A_wqkv: jax.Array,
    A_wo: jax.Array,
    B_x: jax.Array,
    B_w1: jax.Array,
    B_b1: jax.Array,
    B_w2: jax.Array,
    B_b2: jax.Array,
):
    B, S, D = A_x.shape
    F = B_w1.shape[1]
    assert B == 1
    x = A_x.reshape(S, D)
    b1 = B_b1.reshape(1, F)
    b2 = B_b2.reshape(1, D)
    n1 = S // TM1
    any_spec = pl.BlockSpec(memory_space=pl.ANY)
    out = pl.pallas_call(
        functools.partial(_kernel, S=S, D=D, F=F),
        out_shape=jax.ShapeDtypeStruct((S, D), A_x.dtype),
        in_specs=[any_spec] * 7,
        out_specs=any_spec,
        scratch_shapes=[
            pltpu.VMEM((S, D), BF),
            pltpu.VMEM((D, 3 * D), BF),
            pltpu.VMEM((D, D), BF),
            pltpu.VMEM((D, F), BF),
            pltpu.VMEM((1, F), BF),
            pltpu.VMEM((F, D), BF),
            pltpu.VMEM((1, D), BF),
            pltpu.VMEM((2 * D, D), BF),
            pltpu.VMEM((D // 128, S, 128), BF),
            pltpu.VMEM((S // 128, D, 128), BF),
            pltpu.VMEM((S // 128, D, 128), BF),
            pltpu.VMEM((2, S // 128, 128, 128), BF),
            pltpu.VMEM((D, S), F32),
            pltpu.VMEM((S, 128), F32),
            pltpu.VMEM((2, TM3, D), BF),
            pltpu.SemaphoreType.DMA((1 + n1 + 5,)),
            pltpu.SemaphoreType.DMA((2,)),
        ],
        compiler_params=pltpu.CompilerParams(vmem_limit_bytes=100 * 1024 * 1024),
    )(x, A_wqkv, A_wo, B_w1, b1, B_w2, b2)
    return out.reshape(B, S, D)
```

```python
import functools
import math

import jax
import jax.numpy as jnp
from jax import lax
import jax.experimental.pallas as pl
import jax.experimental.pallas.tpu as pltpu

BF = jnp.bfloat16
F32 = jnp.float32
U32 = jnp.uint32

H = 32
LN_EPS = 1e-5
LOG2E = 1.4426950408889634

TM1 = 512
TM3 = 256

NSTR = 4
LAGU = 14
DL = 170
VL = 140
PLD = 40
NR = 4

SAFE_B = 60.0
SAFE_V_HI = 2.0 ** 40
SAFE_V_LO = 2.0 ** -40


def _nt(a, b):
    return lax.dot_general(a, b, (((1,), (1,)), ((), ())), preferred_element_type=F32)


def _layernorm(x):
    m = jnp.mean(x, axis=-1, keepdims=True)
    xc = x - m
    v = jnp.mean(xc * xc, axis=-1, keepdims=True)
    return xc * lax.rsqrt(v + LN_EPS)


def _gelu(x):
    c = math.sqrt(2.0 / math.pi)
    return 0.5 * x * (1.0 + jnp.tanh(c * (x + 0.044715 * (x * x * x))))


def _pack_i(a, b):
    return pltpu.pack_elementwise([a, b], packed_dtype=BF).astype(U32)


def _pack_rows_interleaved(x):
    n, w = x.shape
    x4 = x.reshape(n // 16, 2, 8, w)
    return _pack_i(x4[:, 0], x4[:, 1]).reshape(n // 2, w)


def _attention_events(nq, nlt):
    nt = nq * nlt
    events = []
    defer = {}
    period = 0
    for b in range(NSTR):
        units = [(n // nlt, n % nlt, i) for n in range(nt) for i in range(7)]
        tot = len(units)
        lagu = LAGU + 2 * b
        pts = []
        for n in range(nt):
            pos = 7 * (n + 1) + lagu
            pts.append((pos - tot, 1, n) if pos >= tot else (pos, 0, n))
        pts.sort()
        defer[b] = [p[2] for p in pts if p[1]]
        cuts = sorted(set([0, tot] + [p[0] for p in pts] + [7 * nlt * (q + 1) for q in range(nq)]))
        tm = 0
        pi = 0
        tpv = {}
        for lo, hi in zip(cuts, cuts[1:] + [None]):
            while pi < len(pts) and pts[pi][0] == lo:
                _, df, n = pts[pi]
                events.append((tm - PLD, 1, b, 'pvld', df, n))
                events.append((tm, 2, b, 'pv', df, n))
                tpv[n] = (tm, df)
                tm += 16
                pi += 1
            if hi is None:
                break
            events.append((tm, 2, b, 'qk', tuple(units[lo:hi])))
            for r in range(lo, hi):
                events.append((tm + (r - lo) * 16 + DL, 0, b, 'post', units[r]))
            tm += (hi - lo) * 16
        period = tm
        for n in range(nt):
            t, df = tpv[n]
            events.append((t + (period if df else 0) - VL, 0, b, 'vpu', n))
        events.append((10 ** 9, 0, b, 'save'))
    pre = []
    for x in range(nlt):
        pre += [('kb', x), ('qb', x)]
    for n, (kind, x) in enumerate(pre):
        events.append((400 + (period - 1200) * n // len(pre), 3, 0, kind, x))
    events.sort(key=lambda e: e[:3])
    return events, defer


def _kernel(x_hbm, wqkv_hbm, wo_hbm, w1_hbm, b1_hbm, w2_hbm, b2_hbm, out_hbm,
            x_s, wqkv_s, wo_s, w1_s, b1_s, w2_s, b2_s, wqvt_s, xn0_s,
            kr_s, qt_s, vt_s, kb_a, kb_b, qb_a, qb_b, ar_s, sv_s, ot_s, st_s, out_s,
            sems, osems, *, S, D, F):
    DH = D // H
    NG = D // 128
    HPG = 128 // DH
    NLT = S // 128
    NQ = NLT // NSTR
    n1 = S // TM1
    n3 = S // TM3
    qscale = (DH ** -0.5) * LOG2E
    RING = NSTR * NR * 64
    KU0 = RING
    QU0 = KU0 + H * NLT * 8

    def cp(src, dst, i):
        return pltpu.make_async_copy(src, dst, sems.at[i])

    def wcols(p):
        return cp(wqkv_hbm.at[:, pl.ds(p * D, D)], wqkv_s.at[p], p)

    c_wq, c_wk, c_wv = wcols(0), wcols(1), wcols(2)
    c_x = [cp(x_hbm.at[pl.ds(i * TM1, TM1)], x_s.at[pl.ds(i * TM1, TM1)], 3 + i) for i in range(n1)]
    rest = [(wo_hbm, wo_s), (w1_hbm, w1_s), (b1_hbm, b1_s), (w2_hbm, w2_s), (b2_hbm, b2_s)]
    c_rest = [cp(s_, d_, 3 + n1 + i) for i, (s_, d_) in enumerate(rest)]
    c_x[0].start()
    c_wq.start()
    c_wv.start()
    c_wk.start()
    for c in c_x[1:]:
        c.start()
    for c in c_rest:
        c.start()

    ar_s[0:RING, :] = jnp.zeros((RING, 128), U32)
    sv_s[...] = jnp.zeros(sv_s.shape, F32)

    c_x[0].wait()
    xn0_s[...] = _layernorm(x_s[0:TM1, :].astype(F32))

    ri = lax.broadcasted_iota(jnp.int32, (128, 128), 0)
    ci = lax.broadcasted_iota(jnp.int32, (128, 128), 1)
    eye = jnp.where(ri == ci, 1.0, 0.0).astype(BF)
    for part, (p, c) in enumerate(((0, c_wq), (2, c_wv))):
        c.wait()
        for b in range(NG):
            blk = _nt(eye, wqkv_s[p, :, b * 128:(b + 1) * 128])
            wqvt_s[part, b * 128:(b + 1) * 128, :] = blk.astype(BF)

    hi = lax.broadcasted_iota(jnp.int32, (H, D), 0)
    cj = lax.broadcasted_iota(jnp.int32, (H, D), 1)
    ind = jnp.where(cj // DH == hi, 1.0, 0.0).astype(BF)

    def kb_store(kb_w, u, kk):
        for d in range(DH):
            kb_w[u, d] = jnp.broadcast_to(kk[:, d:d + 1], (16, 128))

    def qb_store(qb_w, lt, qq):
        for d in range(DH):
            qb_w[lt, d] = jnp.broadcast_to(qq[d:d + 1, :], (8, 128))

    qmax = None
    kmax = None
    vmax = None
    nsub = TM1 // 128
    for i in range(n1):
        r0 = i * TM1
        xf = xn0_s[...] if i == 0 else _layernorm(x_s[r0:r0 + TM1, :].astype(F32))
        xn = xf.astype(BF)
        xi = pltpu.bitcast(_pack_rows_interleaved(xf), BF)
        qb = (_nt(wqvt_s[0], xn) * qscale).astype(BF)
        vb = _nt(wqvt_s[1], xi).astype(BF)
        qu = pltpu.bitcast(qb, U32)
        vu = pltpu.bitcast(vb, U32)
        qf = qb.astype(F32)
        for t in range(nsub):
            lt = r0 // 128 + t
            qt_s[lt] = qu[:, t * 128:(t + 1) * 128]
            ar_s[QU0 + lt * (D // 2):QU0 + (lt + 1) * (D // 2), :] = qu[:, t * 128:(t + 1) * 128]
            vt_s[lt] = vu[:, t * 128:(t + 1) * 128]
            qb_store(qb_a, lt, qf[0:DH, t * 128:(t + 1) * 128])
        if i == 0:
            c_wk.wait()
            for c in c_x[1:]:
                c.wait()
            xn = xn0_s[...].astype(BF)
        kb = jnp.dot(xn, wqkv_s[1], preferred_element_type=F32).astype(BF)
        ku = pltpu.bitcast(kb, U32)
        kf = kb.astype(F32)
        for g in range(NG):
            kg = ku[:, g * 128:(g + 1) * 128]
            for jj in range(HPG):
                h = g * HPG + jj
                kr = kg if jj == 0 else pltpu.roll(kg, 128 - jj * DH, 1)
                kr_s[h, r0 // 2:(r0 + TM1) // 2, :] = kr
                for t in range(nsub):
                    lt = r0 // 128 + t
                    row = KU0 + (h * NLT + lt) * 8
                    ar_s[row:row + 8, :] = kr[t * 64 + 56:t * 64 + 64]
        for t in range(nsub):
            kb_store(kb_a, r0 // 128 + t, kf[t * 128 + 112:(t + 1) * 128, 0:128])
        q2 = qf * qf
        q2 = functools.reduce(jnp.maximum, [q2[:, t * 128:(t + 1) * 128] for t in range(nsub)])
        qn = jnp.dot(ind, q2.astype(BF), preferred_element_type=F32)
        qmax = qn if qmax is None else jnp.maximum(qmax, qn)
        k2 = kf * kf
        k2 = functools.reduce(jnp.maximum, [k2[t * 128:(t + 1) * 128] for t in range(nsub)])
        kn = _nt(ind, k2.astype(BF))
        kmax = kn if kmax is None else jnp.maximum(kmax, kn)
        va = jnp.abs(vb.astype(F32)).reshape(D // 8, 8, TM1).max(axis=0)
        vmax = va if vmax is None else jnp.maximum(vmax, va)

    qh = jnp.max(qmax, axis=1, keepdims=True)
    kh = jnp.max(kmax, axis=1, keepdims=True)
    b2max = jnp.max(qh * kh) * 1.05
    vm = jnp.max(vmax)
    safe = jnp.logical_and(b2max <= SAFE_B * SAFE_B,
                           jnp.logical_and(vm <= SAFE_V_HI, vm >= SAFE_V_LO))

    events, defer = _attention_events(NQ, NLT)

    def srow(b, n, i):
        return ((b * NR + n % NR) * 8 + i) * 8

    def finish(acc, l8):
        return acc / jnp.sum(l8, axis=0, keepdims=True)

    def fast_head(h, zero, kb_r, qb_r, kb_w, qb_w):
        nz = 6
        zs = [zero * (i + 2) for i in range(nz)]
        cnt = [0]

        def nzero():
            cnt[0] += 1
            return zs[cnt[0] % nz]

        zrow = zero * 8
        r0 = pl.multiple_of(h * 8, 8)
        ro = pl.multiple_of(h * DH, DH)
        hn = jnp.minimum(h + 1, H - 1)
        hp = jnp.maximum(h - 1, 0)
        r0p = pl.multiple_of(hp * 8, 8)
        rop = pl.multiple_of(hp * DH, DH)
        sval, accs, ls, pld = {}, {}, {}, {}

        def stage(b, n, i, p0, p1):
            lt = (n // NLT) * NSTR + b
            ls[lt] = p0 if lt not in ls else ls[lt] + p0
            ls[lt] = ls[lt] + p1
            row = srow(b, n, i)
            ar_s[row:row + 8, :] = _pack_i(p0, p1)

        for ev in events:
            b, kind = ev[2], ev[3]
            if kind == 'qk':
                us = ev[4]
                lt = us[0][0] * NSTR + b
                runs = []
                for (_, j, i) in us:
                    r = j * 8 + i
                    if runs and runs[-1][1] == r:
                        runs[-1][1] = r + 1
                    else:
                        runs.append([r, r + 1])
                parts = [kr_s[h, a * 8:c * 8, :] for a, c in runs]
                kc = parts[0] if len(parts) == 1 else jnp.concatenate(parts, axis=0)
                kc = pltpu.bitcast(kc, BF)[:, :DH]
                q = pltpu.bitcast(qt_s[lt, pl.ds(r0, 8), :], BF)
                s = jnp.dot(kc, q, preferred_element_type=F32)
                for n, u_ in enumerate(us):
                    sval[(b, u_)] = s[n * 16:(n + 1) * 16]
            elif kind == 'post':
                qi, j, i = ev[4]
                p = jnp.exp2(sval.pop((b, ev[4])))
                stage(b, qi * NLT + j, i, p[:8], p[8:])
            elif kind == 'vpu':
                n = ev[4]
                lt = (n // NLT) * NSTR + b
                kb = kb_r[nzero() + n % NLT].reshape(DH, 2, 8, 128)
                qv = qb_r[nzero() + lt].reshape(DH, 1, 8, 128)
                p = jnp.exp2(jnp.sum(kb * qv, axis=0))
                stage(b, n, 7, p[0], p[1])
            elif kind == 'pvld':
                df, n = ev[4:]
                pld[(b, n)] = ar_s[pl.ds(pl.multiple_of(zrow + srow(b, n, 0), 8), 64), :]
            elif kind == 'pv':
                df, n = ev[4:]
                j = n % NLT
                lt = (n // NLT) * NSTR + b
                pt = pltpu.bitcast(pld.pop((b, n)), BF)
                vt = pltpu.bitcast(vt_s[j, pl.ds(r0p if df else r0, 8), :], BF)
                key = (df, lt)
                if key not in accs:
                    accs[key] = sv_s[b if df else NSTR, 0:DH, :]
                accs[key] = accs[key] + jnp.dot(vt, pt, preferred_element_type=F32)
                if j == NLT - 1:
                    l8 = sv_s[b, DH:DH + 8, :] if df else ls[lt]
                    ot_s[pl.ds(rop if df else ro, DH), lt * 128:(lt + 1) * 128] = finish(accs[key], l8)
            elif kind == 'save':
                lt = (NQ - 1) * NSTR + b
                sv_s[b, 0:DH, :] = accs[(0, lt)]
                sv_s[b, DH:DH + 8, :] = ls[lt]
            elif kind == 'kb':
                row = pl.multiple_of(zrow + KU0 + (hn * NLT + ev[4]) * 8, 8)
                kb_store(kb_w, ev[4], pltpu.bitcast(ar_s[pl.ds(row, 8), :], BF).astype(F32))
            elif kind == 'qb':
                row = pl.multiple_of(zrow + QU0 + ev[4] * (D // 2) + hn * 8, 8)
                qb_store(qb_w, ev[4], pltpu.bitcast(ar_s[pl.ds(row, 8), :], BF).astype(F32))

    def fast_body(h, zero):
        @pl.when(h % 2 == 0)
        def _():
            fast_head(h, zero, kb_a, qb_a, kb_b, qb_b)

        @pl.when(h % 2 == 1)
        def _():
            fast_head(h, zero, kb_b, qb_b, kb_a, qb_a)

        return zero * h

    def slow_head(h, carry):
        r0 = pl.multiple_of(h * 8, 8)
        ro = pl.multiple_of(h * DH, DH)

        def qblock(qi, c2):
            q = pltpu.bitcast(qt_s[qi, pl.ds(r0, 8), :], BF)
            kc = pltpu.bitcast(kr_s[h], BF)[:, :DH]
            st_s[...] = jnp.dot(kc, q, preferred_element_type=F32)
            m = jnp.max(st_s[...], axis=0, keepdims=True)
            acc = jnp.zeros((DH, 128), F32)
            l = jnp.zeros((1, 128), F32)
            for kt in range(NLT):
                p = jnp.exp2(st_s[kt * 128:(kt + 1) * 128, :] - m)
                l = l + jnp.sum(p, axis=0, keepdims=True)
                vt = pltpu.bitcast(vt_s[kt, pl.ds(r0, 8), :], BF)
                pt = pltpu.bitcast(_pack_rows_interleaved(p), BF)
                acc = acc + jnp.dot(vt, pt, preferred_element_type=F32)
            q0 = pl.multiple_of(qi * 128, 128)
            ot_s[pl.ds(ro, DH), pl.ds(q0, 128)] = acc / l
            return c2

        lax.fori_loop(0, NLT, qblock, 0)
        return carry

    @pl.when(safe)
    def _():
        sv_s[0:NSTR, DH:DH + 8, :] = jnp.ones((NSTR, 8, 128), F32)
        lax.fori_loop(0, H, fast_body, 0)
        for b in range(NSTR):
            lt = (NQ - 1) * NSTR + b
            acc = sv_s[b, 0:DH, :]
            for n in defer[b]:
                row = srow(b, n, 0)
                pt = pltpu.bitcast(ar_s[row:row + 64, :], BF)
                vt = pltpu.bitcast(vt_s[n % NLT, (H - 1) * 8:H * 8, :], BF)
                acc = acc + jnp.dot(vt, pt, preferred_element_type=F32)
            ot_s[(H - 1) * DH:H * DH, lt * 128:(lt + 1) * 128] = finish(acc, sv_s[b, DH:DH + 8, :])

    @pl.when(jnp.logical_not(safe))
    def _():
        lax.fori_loop(0, H, slow_head, 0)

    for c in c_rest:
        c.wait()

    def ocp(i):
        return pltpu.make_async_copy(out_s.at[pl.ds(i * TM3, TM3)], out_hbm.at[pl.ds(i * TM3, TM3)], osems.at[i])

    def stage_a(i):
        r0 = i * TM3
        o = ot_s[:, r0:r0 + TM3].T.astype(BF)
        attn = jnp.dot(o, wo_s[...], preferred_element_type=F32)
        h = x_s[r0:r0 + TM3, :].astype(F32) + attn
        return h, _layernorm(h).astype(BF)

    b1v = b1_s[...].astype(F32).reshape(1, F)
    b2v = b2_s[...].astype(F32).reshape(1, D)
    pend = [stage_a(0), stage_a(1)]
    for i in range(n3):
        r0 = i * TM3
        h, hn_ = pend.pop(0)
        u = jnp.dot(hn_, w1_s[...], preferred_element_type=F32) + b1v
        u = _gelu(u).astype(BF)
        if i + 2 < n3:
            pend.append(stage_a(i + 2))
        y = jnp.dot(u, w2_s[...], preferred_element_type=F32) + b2v
        out_s[r0:r0 + TM3, :] = (h + y).astype(out_s.dtype)
        ocp(i).start()
    for i in range(n3):
        ocp(i).wait()


@jax.jit
def pallas_sequential_preLN__softmax_full_mha__dense_activation_gelu__prompt_kernel(
    A_x: jax.Array,
    A_wqkv: jax.Array,
    A_wo: jax.Array,
    B_x: jax.Array,
    B_w1: jax.Array,
    B_b1: jax.Array,
    B_w2: jax.Array,
    B_b2: jax.Array,
):
    B, S, D = A_x.shape
    F = B_w1.shape[1]
    assert B == 1 and D // H == 16 and S % (128 * NSTR) == 0
    x = A_x.reshape(S, D)
    n1 = S // TM1
    nlt = S // 128
    dh = D // H
    arows = NSTR * NR * 64 + H * nlt * 8 + nlt * (D // 2)
    any_spec = pl.BlockSpec(memory_space=pl.ANY)
    out = pl.pallas_call(
        functools.partial(_kernel, S=S, D=D, F=F),
        out_shape=jax.ShapeDtypeStruct((S, D), A_x.dtype),
        in_specs=[any_spec] * 7,
        out_specs=any_spec,
        scratch_shapes=[
            pltpu.VMEM((S, D), BF),
            pltpu.VMEM((3, D, D), BF),
            pltpu.VMEM((D, D), BF),
            pltpu.VMEM((D, F), BF),
            pltpu.VMEM((F,), BF),
            pltpu.VMEM((F, D), BF),
            pltpu.VMEM((D,), BF),
            pltpu.VMEM((2, D, D), BF),
            pltpu.VMEM((TM1, D), F32),
            pltpu.VMEM((H, S // 2, 128), U32),
            pltpu.VMEM((nlt, D // 2, 128), U32),
            pltpu.VMEM((nlt, D // 2, 128), U32),
            pltpu.VMEM((nlt, dh, 16, 128), F32),
            pltpu.VMEM((nlt, dh, 16, 128), F32),
            pltpu.VMEM((nlt, dh, 8, 128), F32),
            pltpu.VMEM((nlt, dh, 8, 128), F32),
            pltpu.VMEM((arows, 128), U32),
            pltpu.VMEM((NSTR + 1, dh + 8, 128), F32),
            pltpu.VMEM((D, S), F32),
            pltpu.VMEM((S, 128), F32),
            pltpu.VMEM((S, D), BF),
            pltpu.SemaphoreType.DMA((3 + n1 + 5,)),
            pltpu.SemaphoreType.DMA((S // TM3,)),
        ],
        compiler_params=pltpu.CompilerParams(vmem_limit_bytes=100 * 1024 * 1024),
    )(x, A_wqkv, A_wo, B_w1, B_b1, B_w2, B_b2)
    return out.reshape(B, S, D)
```

```python
import functools
import math

import jax
import jax.numpy as jnp
from jax import lax
import jax.experimental.pallas as pl
import jax.experimental.pallas.tpu as pltpu

BF = jnp.bfloat16
F32 = jnp.float32
U32 = jnp.uint32

H = 32
LN_EPS = 1e-5
LOG2E = 1.4426950408889634

TM1 = 512
TM3 = 256

NSTR = 4
LAGU = 14
DL = 170
VL = 140
PLD = 48
GD = 140
KS = 4
QS = 2
P0 = 200
P1 = 300
NR = 4

SAFE_B = 60.0
SAFE_V_HI = 2.0 ** 40
SAFE_V_LO = 2.0 ** -40


def _nt(a, b):
    return lax.dot_general(a, b, (((1,), (1,)), ((), ())), preferred_element_type=F32)


def _layernorm(x):
    m = jnp.mean(x, axis=-1, keepdims=True)
    xc = x - m
    v = jnp.mean(xc * xc, axis=-1, keepdims=True)
    return xc * lax.rsqrt(v + LN_EPS)


def _gelu(x):
    c = math.sqrt(2.0 / math.pi)
    return 0.5 * x * (1.0 + jnp.tanh(c * (x + 0.044715 * (x * x * x))))


def _check_events(events, nq, nlt):
    nt = nq * nlt
    assert nt % NR == 0
    ring = {}
    for blk in range(2):
        over = set()
        for e in events:
            b, kind = e[2], e[3]
            if kind == 'post':
                n = e[4][0] * nlt + e[4][1]
                assert ring.get((b, n % NR, e[4][2])) is None
                ring[(b, n % NR, e[4][2])] = (blk, n)
            elif kind == 'vpu':
                df, n = e[4:]
                if df:
                    assert ('kb', n % nlt) not in over and ('qb', (n // nlt) * NSTR + b) not in over
                assert ring.get((b, n % NR, 7)) is None
                ring[(b, n % NR, 7)] = (blk - df, n)
            elif kind == 'pvld':
                df, n = e[4:]
                for i in range(8):
                    got = ring.pop((b, n % NR, i), None)
                    assert blk - df < 0 or got == (blk - df, n)
            elif kind in ('kb', 'qb'):
                over.add((kind, e[4]))


def _attention_events(nq, nlt):
    nt = nq * nlt
    events = []
    defer = {}
    gdefer = []
    period = 0
    for b in range(NSTR):
        units = [(n // nlt, n % nlt, i) for n in range(nt) for i in range(7)]
        tot = len(units)
        lagu = LAGU + 2 * b
        pts = []
        for n in range(nt):
            pos = 7 * (n + 1) + lagu
            pts.append((pos - tot, 1, n) if pos >= tot else (pos, 0, n))
        pts.sort()
        defer[b] = [p[2] for p in pts if p[1]]
        cuts = sorted(set([0, tot] + [p[0] for p in pts] + [7 * nlt * (q + 1) for q in range(nq)]))
        tm = 0
        pi = 0
        tpv = {}
        for lo, hi in zip(cuts, cuts[1:] + [None]):
            while pi < len(pts) and pts[pi][0] == lo:
                _, df, n = pts[pi]
                events.append((tm - PLD, 1, b, 'pvld', df, n))
                events.append((tm, 2, b, 'pv', df, n))
                tpv[n] = (tm, df)
                tm += 16
                pi += 1
            if hi is None:
                break
            events.append((tm, 2, b, 'qk', tuple(units[lo:hi])))
            for r in range(lo, hi):
                events.append((tm + (r - lo) * 16 + DL, 0, b, 'post', units[r]))
            tm += (hi - lo) * 16
        period = tm
        for n in range(nt):
            t, df = tpv[n]
            tg = t + (period if df else 0) - VL
            if tg >= period + GD:
                events.append((tg - period, 0, b, 'vpu', 1, n))
                gdefer.append((b, n))
            else:
                events.append((tg, 0, b, 'vpu', 0, n))
        events.append((10 ** 9, 0, b, 'save'))
    pre = []
    for x in range(nlt):
        pre += [('kb', x, i) for i in range(KS)] + [('qb', x, i) for i in range(QS)]
    for n, e in enumerate(pre):
        events.append((P0 + (period - P0 - P1) * n // len(pre), 3, 0) + e)
    events.sort(key=lambda e: e[:3])
    _check_events(events, nq, nlt)
    return events, defer, gdefer


def _kernel(x_hbm, wqkv_hbm, wo_hbm, w1_hbm, b1_hbm, w2_hbm, b2_hbm, out_hbm,
            x_s, wqkv_s, wo_s, w1_s, w2_s, wqvt_s, xn0_s, q2_s, k2_s, v8_s,
            kr_s, qt_s, vt_s, kb_a, kb_b, qb_a, qb_b, ar_s, sv_s, ot_s, st_s, out_s, h_s, hn_s, b1_s, b2_s,
            sems, osems, *, S, D, F):
    DH = D // H
    NG = D // 128
    HPG = 128 // DH
    NLT = S // 128
    NQ = NLT // NSTR
    n1 = S // TM1
    n3 = S // TM3
    qscale = (DH ** -0.5) * LOG2E
    RING = NSTR * NR * 128
    KU0 = RING
    QU0 = KU0 + (H // 2) * NLT * 16

    def cp(src, dst, i):
        return pltpu.make_async_copy(src, dst, sems.at[i])

    def wcols(p):
        return cp(wqkv_hbm.at[:, pl.ds(p * D, D)], wqkv_s.at[p], p)

    c_wq, c_wk, c_wv = wcols(0), wcols(1), wcols(2)
    c_x = [cp(x_hbm.at[pl.ds(i * TM1, TM1)], x_s.at[pl.ds(i * TM1, TM1)], 3 + i) for i in range(n1)]
    rest = [(wo_hbm, wo_s), (w1_hbm, w1_s), (b1_hbm, b1_s), (w2_hbm, w2_s), (b2_hbm, b2_s)]
    c_rest = [cp(s_, d_, 3 + n1 + i) for i, (s_, d_) in enumerate(rest)]
    c_x[0].start()
    c_wq.start()
    c_wk.start()
    c_wv.start()
    for c in c_x[1:]:
        c.start()

    events, defer, gdefer = _attention_events(NQ, NLT)
    ar_s[0:RING, :] = jnp.zeros((RING, 128), BF)
    sv_s[...] = jnp.zeros(sv_s.shape, F32)
    sv_s[0:NSTR, DH:DH + 8, :] = jnp.ones((NSTR, 8, 128), F32)
    for u in sorted(set(n % NLT for _, n in gdefer)):
        kb_b[u] = jnp.zeros((DH, 16, 128), F32)
    for lt in sorted(set((n // NLT) * NSTR + b for b, n in gdefer)):
        qb_b[lt] = jnp.zeros((DH, 8, 128), F32)

    c_x[0].wait()
    xn0_s[...] = _layernorm(x_s[0:TM1, :].astype(F32)).astype(BF)

    def transpose_w(part, p):
        wqvt_s[part * D:(part + 1) * D, :] = wqkv_s[p].T

    c_wq.wait()
    transpose_w(0, 0)

    hi = lax.broadcasted_iota(jnp.int32, (H, D), 0)
    cj = lax.broadcasted_iota(jnp.int32, (H, D), 1)
    ind = jnp.where(cj // DH == hi, 1.0, 0.0).astype(BF)

    def kb_store(kb_w, u, kk, lo, ds=range(DH)):
        for d in ds:
            kb_w[u, d] = jnp.broadcast_to(kk[:, lo + d:lo + d + 1], (16, 128))

    def qb_store(qb_w, lt, qq, ds=range(DH)):
        for d in ds:
            qb_w[lt, d] = jnp.broadcast_to(qq[d:d + 1, :], (8, 128))

    nsub = TM1 // 128
    stats = {'q': None, 'k': None, 'v': None}

    def upd(name, val):
        stats[name] = val if stats[name] is None else jnp.maximum(stats[name], val)

    def norm_dots(q2, k2):
        upd('q', jnp.dot(ind, q2, preferred_element_type=F32))
        upd('k', _nt(ind, k2))

    def v_part(xn, r0, m0, m1):
        vb = _nt(wqvt_s[D + m0:D + m1, :], xn).astype(BF)
        vu = pltpu.bitcast(vb, U32)
        for t in range(nsub):
            vt_s[m0 // DH:m1 // DH, r0 // 128 + t] = (
                vu[:, t * 128:(t + 1) * 128].reshape((m1 - m0) // DH, 8, 128))
        upd('v', jnp.abs(vb.astype(F32)).reshape((m1 - m0) // 8, 8, TM1).max(axis=0))

    for i in range(n1):
        r0 = i * TM1
        xn = xn0_s[...] if i == 0 else _layernorm(x_s[r0:r0 + TM1, :].astype(F32)).astype(BF)
        qb = (_nt(wqvt_s[0:D, :], xn) * qscale).astype(BF)
        qu = pltpu.bitcast(qb, U32)
        qf = qb.astype(F32)
        for t in range(nsub):
            lt = r0 // 128 + t
            qt_s[:, lt] = qu[:, t * 128:(t + 1) * 128].reshape(H, 8, 128)
            for hh in range(H):
                row = QU0 + (hh * NLT + lt) * 16
                ar_s[row:row + 16, :] = qb[hh * DH:(hh + 1) * DH, t * 128:(t + 1) * 128]
            qb_store(qb_a, lt, qf[0:DH, t * 128:(t + 1) * 128])
        q2 = qf * qf
        q2 = functools.reduce(jnp.maximum, [q2[:, t * 128:(t + 1) * 128] for t in range(nsub)]).astype(BF)
        if i == 0:
            q2_s[...] = q2
            c_wk.wait()
            c_wv.wait()
            xn = xn0_s[...]
        kb = jnp.dot(xn, wqkv_s[1], preferred_element_type=F32).astype(BF)
        ku = pltpu.bitcast(kb, U32)
        kf = kb.astype(F32)
        for g in range(NG):
            kg = ku[:, g * 128:(g + 1) * 128]
            for jj in range(HPG // 2):
                hp2 = g * (HPG // 2) + jj
                kr = kg if jj == 0 else pltpu.roll(kg, 128 - jj * 2 * DH, 1)
                kr_s[hp2, r0 // 2:(r0 + TM1) // 2, :] = kr
                for t in range(nsub):
                    row = KU0 + (hp2 * NLT + r0 // 128 + t) * 16
                    ar_s[row:row + 16, :] = pltpu.bitcast(kr[t * 64 + 56:t * 64 + 64], BF)
        for t in range(nsub):
            kb_store(kb_a, r0 // 128 + t, kf[t * 128 + 112:(t + 1) * 128, 0:128], 0)
        k2 = kf * kf
        k2 = functools.reduce(jnp.maximum, [k2[t * 128:(t + 1) * 128] for t in range(nsub)]).astype(BF)
        if i == 0:
            transpose_w(1, 2)
        v_part(xn, r0, 0, D // 2)
        if i == 0:
            k2_s[...] = k2
            v8_s[...] = stats['v']
            for c in c_x[1:]:
                c.wait()
            for c in c_rest:
                c.start()
            xn = xn0_s[...]
            q2 = q2_s[...]
            k2 = k2_s[...]
            stats['v'] = v8_s[...]
        norm_dots(q2, k2)
        v_part(xn, r0, D // 2, D)

    qmax, kmax, vmax = stats['q'], stats['k'], stats['v']
    qh = jnp.max(qmax, axis=1, keepdims=True)
    kh = jnp.max(kmax, axis=1, keepdims=True)
    b2max = jnp.max(qh * kh) * 1.05
    vm = jnp.max(vmax)
    safe = jnp.logical_and(b2max <= SAFE_B * SAFE_B,
                           jnp.logical_and(vm <= SAFE_V_HI, vm >= SAFE_V_LO))


    def srow(b, n, i):
        return ((b * NR + n % NR) * 8 + i) * 16

    def finish(acc, l8):
        return acc / jnp.sum(l8, axis=0, keepdims=True)

    def vpu_scores(kb, qv):
        return jnp.exp2(jnp.sum(kb.reshape(DH, 2, 8, 128) * qv.reshape(DH, 1, 8, 128), axis=0)).reshape(16, 128)

    def fast_head(h, zero, odd, kb_r, qb_r, kb_w, qb_w):
        nz = 6
        zs = [zero * (i + 2) for i in range(nz)]
        cnt = [0]

        def nzero():
            cnt[0] += 1
            return zs[cnt[0] % nz]

        zrow = zero * 16
        h2 = lax.shift_right_logical(h, 1)
        ro = pl.multiple_of(h * DH, DH)
        hn = jnp.minimum(h + 1, H - 1)
        hn2 = lax.shift_right_logical(hn, 1)
        hp = jnp.maximum(h - 1, 0)
        rop = pl.multiple_of(hp * DH, DH)
        sval, accs, ls, pld = {}, {}, {}, {}

        ring = ar_s.bitcast(U32).at[pl.ds(pl.multiple_of(zero * 8, 8), RING // 2)]
        ksrc = ar_s.at[pl.ds(pl.multiple_of(zrow + KU0 + hn2 * (NLT * 16), 16), NLT * 16)]
        qsrc = ar_s.at[pl.ds(pl.multiple_of(zrow + QU0 + hn * (NLT * 16), 16), NLT * 16)]
        for b in range(NSTR):
            ls[(1, (NQ - 1) * NSTR + b)] = sv_s[b, DH:DH + 8, :]

        def stage(b, n, i, p, df=0):
            lt = (df, (n // NLT) * NSTR + b)
            ls[lt] = p[:8] if lt not in ls else ls[lt] + p[:8]
            ls[lt] = ls[lt] + p[8:]
            row = srow(b, n, i)
            ar_s[row:row + 16, :] = p.astype(BF)

        for ev in events:
            b, kind = ev[2], ev[3]
            if kind == 'qk':
                us = ev[4]
                lt = us[0][0] * NSTR + b
                runs = []
                for (_, j, i) in us:
                    r = j * 8 + i
                    if runs and runs[-1][1] == r:
                        runs[-1][1] = r + 1
                    else:
                        runs.append([r, r + 1])
                parts = [kr_s[h2, a * 8:c * 8, :] for a, c in runs]
                kc = parts[0] if len(parts) == 1 else jnp.concatenate(parts, axis=0)
                q = qt_s[h, lt]
                if odd:
                    q = jnp.concatenate([jnp.zeros_like(q), q], axis=0)
                kc = pltpu.bitcast(kc, BF)[:, :(2 * DH if odd else DH)]
                s = jnp.dot(kc, pltpu.bitcast(q, BF), preferred_element_type=F32)
                for n, u_ in enumerate(us):
                    sval[(b, u_)] = s[n * 16:(n + 1) * 16]
            elif kind == 'post':
                qi, j, i = ev[4]
                p = jnp.exp2(sval.pop((b, ev[4])))
                stage(b, qi * NLT + j, i, p)
            elif kind == 'vpu':
                df, n = ev[4:]
                lt = (n // NLT) * NSTR + b
                if df:
                    p = vpu_scores(kb_w[n % NLT], qb_w[lt])
                else:
                    p = vpu_scores(kb_r[nzero() + n % NLT], qb_r[nzero() + lt])
                stage(b, n, 7, p, df)
            elif kind == 'pvld':
                df, n = ev[4:]
                row = srow(b, n, 0) // 2
                pld[(b, n)] = pltpu.bitcast(ring[row:row + 64, :], BF)
            elif kind == 'pv':
                df, n = ev[4:]
                j = n % NLT
                lt = (n // NLT) * NSTR + b
                pt = pld.pop((b, n))
                vt = pltpu.bitcast(vt_s[hp if df else h, j], BF)
                key = (df, lt)
                if key not in accs:
                    accs[key] = sv_s[b if df else NSTR, 0:DH, :]
                accs[key] = accs[key] + jnp.dot(vt, pt, preferred_element_type=F32)
                if j == NLT - 1:
                    ot_s[pl.ds(rop if df else ro, DH), lt * 128:(lt + 1) * 128] = finish(accs[key], ls[key])
            elif kind == 'save':
                lt = (NQ - 1) * NSTR + b
                sv_s[b, 0:DH, :] = accs[(0, lt)]
                sv_s[b, DH:DH + 8, :] = ls[(0, lt)]
            elif kind == 'kb':
                row = ev[4] * 16
                ds = range(ev[5] * DH // KS, (ev[5] + 1) * DH // KS)
                kb_store(kb_w, ev[4], ksrc[row:row + 16, :].astype(F32), 0 if odd else DH, ds)
            elif kind == 'qb':
                row = ev[4] * 16
                ds = range(ev[5] * DH // QS, (ev[5] + 1) * DH // QS)
                qb_store(qb_w, ev[4], qsrc[row:row + 16, :].astype(F32), ds)

    def fast_body(h2, zero):
        @pl.when(zero == 0)
        def _():
            fast_head(2 * h2, zero, False, kb_a, qb_a, kb_b, qb_b)

        fast_head(2 * h2 + 1, zero, True, kb_b, qb_b, kb_a, qb_a)

        return zero * h2

    def slow_head(h, carry):
        ro = pl.multiple_of(h * DH, DH)

        def qblock(qi, c2):
            q = qt_s[h, qi]
            z = jnp.zeros_like(q)
            q = jnp.where((h & 1) == 1, jnp.concatenate([z, q], axis=0), jnp.concatenate([q, z], axis=0))
            q = pltpu.bitcast(q, BF)
            kc = pltpu.bitcast(kr_s[lax.shift_right_logical(h, 1)], BF)[:, :2 * DH]
            st_s[...] = jnp.dot(kc, q, preferred_element_type=F32)
            m = jnp.max(st_s[...], axis=0, keepdims=True)
            acc = jnp.zeros((DH, 128), F32)
            l = jnp.zeros((1, 128), F32)
            for kt in range(NLT):
                p = jnp.exp2(st_s[kt * 128:(kt + 1) * 128, :] - m)
                l = l + jnp.sum(p, axis=0, keepdims=True)
                vt = pltpu.bitcast(vt_s[h, kt], BF)
                acc = acc + jnp.dot(vt, p.astype(BF), preferred_element_type=F32)
            q0 = pl.multiple_of(qi * 128, 128)
            ot_s[pl.ds(ro, DH), pl.ds(q0, 128)] = acc / l
            return c2

        lax.fori_loop(0, NLT, qblock, 0)
        return carry

    def stage_a(r0, n, h_w, hn_w, w0):
        o = ot_s[:, pl.ds(r0, n)].T.astype(BF)
        attn = jnp.dot(o, wo_s[...], preferred_element_type=F32)
        h = x_s[pl.ds(r0, n), :].astype(F32) + attn
        h_w[w0:w0 + n, :] = h
        hn_w[w0:w0 + n, :] = _layernorm(h).astype(BF)

    def first_a():
        stage_a(0, TM3 // 2, h_s, hn_s, 0)
        stage_a(TM3 // 2, TM3 // 2, h_s, hn_s, TM3 // 2)

    def fast_path():
        lax.fori_loop(0, H // 2, fast_body, 0)
        for b in range(NSTR):
            lt = (NQ - 1) * NSTR + b
            acc = sv_s[b, 0:DH, :]
            l8 = sv_s[b, DH:DH + 8, :]
            for (b_, n) in gdefer:
                if b_ == b:
                    p = vpu_scores(kb_b[n % NLT], qb_b[lt])
                    l8 = l8 + p[:8] + p[8:]
                    ar_s[srow(b, n, 7):srow(b, n, 7) + 16, :] = p.astype(BF)
            for n in defer[b]:
                row = srow(b, n, 0)
                pt = ar_s[row:row + 128, :]
                vt = pltpu.bitcast(vt_s[H - 1, n % NLT], BF)
                acc = acc + jnp.dot(vt, pt, preferred_element_type=F32)
            ot_s[(H - 1) * DH:H * DH, lt * 128:(lt + 1) * 128] = finish(acc, l8)
        first_a()

    def slow_path():
        lax.fori_loop(0, H, slow_head, 0)
        first_a()

    for c in c_rest:
        c.wait()
    lax.cond(safe, fast_path, slow_path)

    def ocp(i, r0, n):
        return pltpu.make_async_copy(out_s.at[pl.ds(r0, n)], out_hbm.at[pl.ds(r0, n)], osems.at[i])

    def ffn(i, prefetch):
        r0 = pl.multiple_of(i * TM3, TM3) if prefetch else i * TM3
        span = 2 * TM3 if prefetch else TM3
        hv = h_s.at[pl.ds(r0, span)]
        hnv = hn_s.at[pl.ds(r0, span)]
        u = jnp.dot(hnv[0:TM3, :], w1_s[...], preferred_element_type=F32)
        u = _gelu(u + b1_s[...].astype(F32).reshape(1, F)).astype(BF)
        if prefetch:
            stage_a(pl.multiple_of(r0 + TM3, TM3), TM3, hv, hnv, TM3)
        b2v = b2_s[...].astype(F32).reshape(1, D)
        nparts = 1 if prefetch else 2
        n = TM3 // nparts
        for t in range(nparts):
            y = jnp.dot(u[t * n:(t + 1) * n], w2_s[...], preferred_element_type=F32) + b2v
            out_s[pl.ds(r0 + t * n, n), :] = (hv[t * n:(t + 1) * n, :] + y).astype(out_s.dtype)
            ocp(i + t, r0 + t * n, n).start()

    def ffn_body(i, c):
        ffn(i, True)
        return c

    lax.fori_loop(0, n3 - 1, ffn_body, 0)
    ffn(n3 - 1, False)
    for i in range(n3 - 1):
        ocp(i, i * TM3, TM3).wait()
    for t in range(2):
        ocp(n3 - 1 + t, (n3 - 1) * TM3 + t * (TM3 // 2), TM3 // 2).wait()


@jax.jit
def pallas_sequential_preLN__softmax_full_mha__dense_activation_gelu__prompt_kernel(
    A_x: jax.Array,
    A_wqkv: jax.Array,
    A_wo: jax.Array,
    B_x: jax.Array,
    B_w1: jax.Array,
    B_b1: jax.Array,
    B_w2: jax.Array,
    B_b2: jax.Array,
):
    B, S, D = A_x.shape
    F = B_w1.shape[1]
    assert B == 1 and D // H == 16 and S % (128 * NSTR) == 0
    x = A_x.reshape(S, D)
    n1 = S // TM1
    nlt = S // 128
    dh = D // H
    arows = NSTR * NR * 128 + (H // 2) * nlt * 16 + nlt * D
    any_spec = pl.BlockSpec(memory_space=pl.ANY)
    out = pl.pallas_call(
        functools.partial(_kernel, S=S, D=D, F=F),
        out_shape=jax.ShapeDtypeStruct((S, D), A_x.dtype),
        in_specs=[any_spec] * 7,
        out_specs=any_spec,
        scratch_shapes=[
            pltpu.VMEM((S, D), BF),
            pltpu.VMEM((3, D, D), BF),
            pltpu.VMEM((D, D), BF),
            pltpu.VMEM((D, F), BF),
            pltpu.VMEM((F, D), BF),
            pltpu.VMEM((2 * D, D), BF),
            pltpu.VMEM((TM1, D), BF),
            pltpu.VMEM((D, 128), BF),
            pltpu.VMEM((128, D), BF),
            pltpu.VMEM((8, TM1), F32),
            pltpu.VMEM((H // 2, S // 2, 128), U32),
            pltpu.VMEM((H, nlt, 8, 128), U32),
            pltpu.VMEM((H, nlt, 8, 128), U32),
            pltpu.VMEM((nlt, dh, 16, 128), F32),
            pltpu.VMEM((nlt, dh, 16, 128), F32),
            pltpu.VMEM((nlt, dh, 8, 128), F32),
            pltpu.VMEM((nlt, dh, 8, 128), F32),
            pltpu.VMEM((arows, 128), BF),
            pltpu.VMEM((NSTR + 1, 32, 128), F32),
            pltpu.VMEM((D, S), F32),
            pltpu.VMEM((S, 128), F32),
            pltpu.VMEM((S, D), BF),
            pltpu.VMEM((S, D), F32),
            pltpu.VMEM((S, D), BF),
            pltpu.VMEM((F,), BF),
            pltpu.VMEM((D,), BF),
            pltpu.SemaphoreType.DMA((3 + n1 + 5,)),
            pltpu.SemaphoreType.DMA((S // TM3 + 1,)),
        ],
        compiler_params=pltpu.CompilerParams(vmem_limit_bytes=100 * 1024 * 1024),
    )(x, A_wqkv, A_wo, B_w1, B_b1, B_w2, B_b2)
    return out.reshape(B, S, D)
```

```python
import functools
import math

import jax
import jax.numpy as jnp
from jax import lax
import jax.experimental.pallas as pl
import jax.experimental.pallas.tpu as pltpu

BF = jnp.bfloat16
F32 = jnp.float32
U32 = jnp.uint32

H = 32
LN_EPS = 1e-5
LOG2E = 1.4426950408889634

TM1 = 512
TM3 = 256

NSTR = 4
LAGU = 14
DL = 170
VL = 144
PLD = 56
GD = 140
KS = 4
QS = 4
P0 = 200
P1 = 300
NR = 4

SAFE_B = 60.0
SAFE_V_HI = 2.0 ** 40
SAFE_V_LO = 2.0 ** -40


def _nt(a, b):
    return lax.dot_general(a, b, (((1,), (1,)), ((), ())), preferred_element_type=F32)


def _layernorm(x):
    m = jnp.mean(x, axis=-1, keepdims=True)
    xc = x - m
    v = jnp.mean(xc * xc, axis=-1, keepdims=True)
    return xc * lax.rsqrt(v + LN_EPS)


def _gelu(x):
    c = math.sqrt(2.0 / math.pi)
    return 0.5 * x * (1.0 + jnp.tanh(c * (x + 0.044715 * (x * x * x))))


def _check_events(events, nq, nlt):
    nt = nq * nlt
    assert nt % NR == 0
    ring = {}
    for blk in range(2):
        over = set()
        for e in events:
            b, kind = e[2], e[3]
            if kind == 'post':
                n = e[4][0] * nlt + e[4][1]
                assert ring.get((b, n % NR, e[4][2])) is None
                ring[(b, n % NR, e[4][2])] = (blk, n)
            elif kind == 'vpu':
                df, n = e[4:]
                if df:
                    assert ('kb', n % nlt) not in over and ('qb', (n // nlt) * NSTR + b) not in over
                assert ring.get((b, n % NR, 7)) is None
                ring[(b, n % NR, 7)] = (blk - df, n)
            elif kind == 'pvld':
                df, n = e[4:]
                for i in range(8):
                    got = ring.pop((b, n % NR, i), None)
                    assert blk - df < 0 or got == (blk - df, n)
            elif kind in ('kb', 'qb'):
                over.add((kind, e[4]))


def _attention_events(nq, nlt):
    nt = nq * nlt
    events = []
    defer = {}
    gdefer = []
    period = 0
    for b in range(NSTR):
        units = [(n // nlt, n % nlt, i) for n in range(nt) for i in range(7)]
        tot = len(units)
        lagu = LAGU + 2 * b
        pts = []
        for n in range(nt):
            pos = 7 * (n + 1) + lagu
            pts.append((pos - tot, 1, n) if pos >= tot else (pos, 0, n))
        pts.sort()
        defer[b] = [p[2] for p in pts if p[1]]
        cuts = sorted(set([0, tot] + [p[0] for p in pts] + [7 * nlt * (q + 1) for q in range(nq)]))
        tm = 0
        pi = 0
        tpv = {}
        for lo, hi in zip(cuts, cuts[1:] + [None]):
            while pi < len(pts) and pts[pi][0] == lo:
                _, df, n = pts[pi]
                events.append((tm - PLD, 1, b, 'pvld', df, n))
                events.append((tm, 2, b, 'pv', df, n))
                tpv[n] = (tm, df)
                tm += 16
                pi += 1
            if hi is None:
                break
            events.append((tm, 2, b, 'qk', tuple(units[lo:hi])))
            for r in range(lo, hi):
                events.append((tm + (r - lo) * 16 + DL, 0, b, 'post', units[r]))
            tm += (hi - lo) * 16
        period = tm
        for n in range(nt):
            t, df = tpv[n]
            tg = t + (period if df else 0) - VL
            if tg >= period + GD:
                events.append((tg - period, 0, b, 'vpu', 1, n))
                gdefer.append((b, n))
            else:
                events.append((tg, 0, b, 'vpu', 0, n))
        events.append((10 ** 9, 0, b, 'save'))
    pre = []
    for x in range(nlt):
        pre += [('kb', x, i) for i in range(KS)] + [('qb', x, i) for i in range(QS)]
    for n, e in enumerate(pre):
        events.append((P0 + (period - P0 - P1) * n // len(pre), 3, 0) + e)
    events.sort(key=lambda e: e[:3])
    _check_events(events, nq, nlt)
    return events, defer, gdefer


def _kernel(x_hbm, wqkv_hbm, wo_hbm, w1_hbm, b1_hbm, w2_hbm, b2_hbm, out_hbm,
            x_s, wqkv_s, wo_s, w1_s, w2_s, wqvt_s, xn0_s, q2_s, k2_s, v8_s,
            kr_s, qt_s, vt_s, kb_a, kb_b, qb_a, qb_b, ar_s, sv_s, ot_s, st_s, out_s, h_s, hn_s, b1_s, b2_s,
            sems, osems, *, S, D, F):
    DH = D // H
    NG = D // 128
    HPG = 128 // DH
    NLT = S // 128
    NQ = NLT // NSTR
    n1 = S // TM1
    n3 = S // TM3
    qscale = (DH ** -0.5) * LOG2E
    RING = NSTR * NR * 128
    KU0 = RING
    QU0 = KU0 + (H // 2) * NLT * 16

    def cp(src, dst, i):
        return pltpu.make_async_copy(src, dst, sems.at[i])

    def wcols(p):
        return cp(wqkv_hbm.at[:, pl.ds(p * D, D)], wqkv_s.at[p], p)

    c_wq, c_wk, c_wv = wcols(0), wcols(1), wcols(2)
    c_x = [cp(x_hbm.at[pl.ds(i * TM1, TM1)], x_s.at[pl.ds(i * TM1, TM1)], 3 + i) for i in range(n1)]
    rest = [(wo_hbm, wo_s), (w1_hbm, w1_s), (b1_hbm, b1_s), (w2_hbm, w2_s), (b2_hbm, b2_s)]
    c_rest = [cp(s_, d_, 3 + n1 + i) for i, (s_, d_) in enumerate(rest)]
    c_x[0].start()
    c_wq.start()
    c_wk.start()
    c_wv.start()
    for c in c_x[1:]:
        c.start()

    events, defer, gdefer = _attention_events(NQ, NLT)
    ar_s[0:RING, :] = jnp.zeros((RING, 128), BF)
    sv_s[...] = jnp.zeros(sv_s.shape, F32)
    sv_s[0:NSTR, DH:DH + 8, :] = jnp.ones((NSTR, 8, 128), F32)
    for u in sorted(set(n % NLT for _, n in gdefer)):
        kb_b[u] = jnp.zeros((DH, 16, 128), F32)
    for lt in sorted(set((n // NLT) * NSTR + b for b, n in gdefer)):
        qb_b[lt] = jnp.zeros((DH, 8, 128), F32)

    c_x[0].wait()
    xn0_s[...] = _layernorm(x_s[0:TM1, :].astype(F32)).astype(BF)

    def transpose_w(part, p):
        wqvt_s[part * D:(part + 1) * D, :] = wqkv_s[p].T

    c_wq.wait()
    transpose_w(0, 0)

    hi = lax.broadcasted_iota(jnp.int32, (H, D), 0)
    cj = lax.broadcasted_iota(jnp.int32, (H, D), 1)
    ind = jnp.where(cj // DH == hi, 1.0, 0.0).astype(BF)

    def kb_store(kb_w, u, kk, lo, ds=range(DH)):
        for d in ds:
            kb_w[u, d] = jnp.broadcast_to(kk[:, lo + d:lo + d + 1], (16, 128))

    def qb_store(qb_w, lt, qq, ds=range(DH)):
        for d in ds:
            qb_w[lt, d] = jnp.broadcast_to(qq[d:d + 1, :], (8, 128))

    nsub = TM1 // 128
    stats = {'q': None, 'k': None, 'v': None}

    def upd(name, val):
        stats[name] = val if stats[name] is None else jnp.maximum(stats[name], val)

    def norm_dots(q2, k2):
        upd('q', jnp.dot(ind, q2, preferred_element_type=F32))
        upd('k', _nt(ind, k2))

    def v_part(xn, r0, m0, m1):
        vb = _nt(wqvt_s[D + m0:D + m1, :], xn).astype(BF)
        vu = pltpu.bitcast(vb, U32)
        for t in range(nsub):
            vt_s[m0 // DH:m1 // DH, r0 // 128 + t] = (
                vu[:, t * 128:(t + 1) * 128].reshape((m1 - m0) // DH, 8, 128))
        upd('v', jnp.abs(vb.astype(F32)).reshape((m1 - m0) // 8, 8, TM1).max(axis=0))

    for i in range(n1):
        r0 = i * TM1
        xn = xn0_s[...] if i == 0 else _layernorm(x_s[r0:r0 + TM1, :].astype(F32)).astype(BF)
        qb = (_nt(wqvt_s[0:D, :], xn) * qscale).astype(BF)
        qu = pltpu.bitcast(qb, U32)
        qf = qb.astype(F32)
        for t in range(nsub):
            lt = r0 // 128 + t
            qt_s[:, lt] = qu[:, t * 128:(t + 1) * 128].reshape(H, 8, 128)
            for hh in range(H):
                row = QU0 + (hh * NLT + lt) * 16
                ar_s[row:row + 16, :] = qb[hh * DH:(hh + 1) * DH, t * 128:(t + 1) * 128]
            qb_store(qb_a, lt, qf[0:DH, t * 128:(t + 1) * 128])
        q2 = qf * qf
        q2 = functools.reduce(jnp.maximum, [q2[:, t * 128:(t + 1) * 128] for t in range(nsub)]).astype(BF)
        if i == 0:
            q2_s[...] = q2
            c_wk.wait()
            c_wv.wait()
            xn = xn0_s[...]
        kb = jnp.dot(xn, wqkv_s[1], preferred_element_type=F32).astype(BF)
        ku = pltpu.bitcast(kb, U32)
        kf = kb.astype(F32)
        for g in range(NG):
            kg = ku[:, g * 128:(g + 1) * 128]
            for jj in range(HPG // 2):
                hp2 = g * (HPG // 2) + jj
                kr = kg if jj == 0 else pltpu.roll(kg, 128 - jj * 2 * DH, 1)
                kr_s[hp2, r0 // 2:(r0 + TM1) // 2, :] = kr
                for t in range(nsub):
                    row = KU0 + (hp2 * NLT + r0 // 128 + t) * 16
                    ar_s[row:row + 16, :] = pltpu.bitcast(kr[t * 64 + 56:t * 64 + 64], BF)
        for t in range(nsub):
            kb_store(kb_a, r0 // 128 + t, kf[t * 128 + 112:(t + 1) * 128, 0:128], 0)
        k2 = kf * kf
        k2 = functools.reduce(jnp.maximum, [k2[t * 128:(t + 1) * 128] for t in range(nsub)]).astype(BF)
        if i == 0:
            transpose_w(1, 2)
        v_part(xn, r0, 0, D // 2)
        if i == 0:
            k2_s[...] = k2
            v8_s[...] = stats['v']
            for c in c_x[1:]:
                c.wait()
            for c in c_rest:
                c.start()
            xn = xn0_s[...]
            q2 = q2_s[...]
            k2 = k2_s[...]
            stats['v'] = v8_s[...]
        norm_dots(q2, k2)
        v_part(xn, r0, D // 2, D)

    qmax, kmax, vmax = stats['q'], stats['k'], stats['v']
    qh = jnp.max(qmax, axis=1, keepdims=True)
    kh = jnp.max(kmax, axis=1, keepdims=True)
    b2max = jnp.max(qh * kh) * 1.05
    vm = jnp.max(vmax)
    safe = jnp.logical_and(b2max <= SAFE_B * SAFE_B,
                           jnp.logical_and(vm <= SAFE_V_HI, vm >= SAFE_V_LO))


    def srow(b, n, i):
        return ((b * NR + n % NR) * 8 + i) * 16

    def finish(acc, l8):
        return acc / jnp.sum(l8, axis=0, keepdims=True)

    def vpu_scores(kb, qv):
        return jnp.exp2(jnp.sum(kb.reshape(DH, 2, 8, 128) * qv.reshape(DH, 1, 8, 128), axis=0)).reshape(16, 128)

    def fast_head(h, zero, odd, kb_r, qb_r, kb_w, qb_w):
        nz = 6
        zs = [zero * (i + 2) for i in range(nz)]
        cnt = [0]

        def nzero():
            cnt[0] += 1
            return zs[cnt[0] % nz]

        zrow = zero * 16
        h2 = lax.shift_right_logical(h, 1)
        ro = pl.multiple_of(h * DH, DH)
        hn = jnp.minimum(h + 1, H - 1)
        hn2 = lax.shift_right_logical(hn, 1)
        hp = jnp.maximum(h - 1, 0)
        rop = pl.multiple_of(hp * DH, DH)
        sval, accs, ls, pld = {}, {}, {}, {}

        ring = ar_s.at[pl.ds(pl.multiple_of(zrow, 16), RING)]
        ksrc = ar_s.at[pl.ds(pl.multiple_of(zrow + KU0 + hn2 * (NLT * 16), 16), NLT * 16)]
        qsrc = ar_s.at[pl.ds(pl.multiple_of(zrow + QU0 + hn * (NLT * 16), 16), NLT * 16)]
        for b in range(NSTR):
            ls[(1, (NQ - 1) * NSTR + b)] = sv_s[b, DH:DH + 8, :]

        def stage(b, n, i, p, df=0):
            lt = (df, (n // NLT) * NSTR + b)
            ls[lt] = p[:8] if lt not in ls else ls[lt] + p[:8]
            ls[lt] = ls[lt] + p[8:]
            row = srow(b, n, i)
            ar_s[row:row + 16, :] = p.astype(BF)

        for ev in events:
            b, kind = ev[2], ev[3]
            if kind == 'qk':
                us = ev[4]
                lt = us[0][0] * NSTR + b
                runs = []
                for (_, j, i) in us:
                    r = j * 8 + i
                    if runs and runs[-1][1] == r:
                        runs[-1][1] = r + 1
                    else:
                        runs.append([r, r + 1])
                parts = [kr_s[h2, a * 8:c * 8, :] for a, c in runs]
                kc = parts[0] if len(parts) == 1 else jnp.concatenate(parts, axis=0)
                q = qt_s[h, lt]
                if odd:
                    q = jnp.concatenate([jnp.zeros_like(q), q], axis=0)
                kc = pltpu.bitcast(kc, BF)[:, :(2 * DH if odd else DH)]
                s = jnp.dot(kc, pltpu.bitcast(q, BF), preferred_element_type=F32)
                for n, u_ in enumerate(us):
                    sval[(b, u_)] = s[n * 16:(n + 1) * 16]
            elif kind == 'post':
                qi, j, i = ev[4]
                p = jnp.exp2(sval.pop((b, ev[4])))
                stage(b, qi * NLT + j, i, p)
            elif kind == 'vpu':
                df, n = ev[4:]
                lt = (n // NLT) * NSTR + b
                if df:
                    p = vpu_scores(kb_w[n % NLT], qb_w[lt])
                else:
                    p = vpu_scores(kb_r[nzero() + n % NLT], qb_r[nzero() + lt])
                stage(b, n, 7, p, df)
            elif kind == 'pvld':
                df, n = ev[4:]
                row = srow(b, n, 0)
                pld[(b, n)] = ring[row:row + 128, :]
            elif kind == 'pv':
                df, n = ev[4:]
                j = n % NLT
                lt = (n // NLT) * NSTR + b
                pt = pld.pop((b, n))
                vt = pltpu.bitcast(vt_s[hp if df else h, j], BF)
                key = (df, lt)
                if key not in accs:
                    accs[key] = sv_s[b if df else NSTR, 0:DH, :]
                accs[key] = accs[key] + jnp.dot(vt, pt, preferred_element_type=F32)
                if j == NLT - 1:
                    ot_s[pl.ds(rop if df else ro, DH), lt * 128:(lt + 1) * 128] = finish(accs[key], ls[key])
            elif kind == 'save':
                lt = (NQ - 1) * NSTR + b
                sv_s[b, 0:DH, :] = accs[(0, lt)]
                sv_s[b, DH:DH + 8, :] = ls[(0, lt)]
            elif kind == 'kb':
                row = ev[4] * 16
                ds = range(ev[5] * DH // KS, (ev[5] + 1) * DH // KS)
                kb_store(kb_w, ev[4], ksrc[row:row + 16, :].astype(F32), 0 if odd else DH, ds)
            elif kind == 'qb':
                row = ev[4] * 16
                ds = range(ev[5] * DH // QS, (ev[5] + 1) * DH // QS)
                qb_store(qb_w, ev[4], qsrc[row:row + 16, :].astype(F32), ds)

    def fast_body(h2, zero):
        @pl.when(zero == 0)
        def _():
            fast_head(2 * h2, zero, False, kb_a, qb_a, kb_b, qb_b)

        fast_head(2 * h2 + 1, zero, True, kb_b, qb_b, kb_a, qb_a)

        return zero * h2

    def slow_head(h, carry):
        ro = pl.multiple_of(h * DH, DH)

        def qblock(qi, c2):
            q = qt_s[h, qi]
            z = jnp.zeros_like(q)
            q = jnp.where((h & 1) == 1, jnp.concatenate([z, q], axis=0), jnp.concatenate([q, z], axis=0))
            q = pltpu.bitcast(q, BF)
            kc = pltpu.bitcast(kr_s[lax.shift_right_logical(h, 1)], BF)[:, :2 * DH]
            st_s[...] = jnp.dot(kc, q, preferred_element_type=F32)
            m = jnp.max(st_s[...], axis=0, keepdims=True)
            acc = jnp.zeros((DH, 128), F32)
            l = jnp.zeros((1, 128), F32)
            for kt in range(NLT):
                p = jnp.exp2(st_s[kt * 128:(kt + 1) * 128, :] - m)
                l = l + jnp.sum(p, axis=0, keepdims=True)
                vt = pltpu.bitcast(vt_s[h, kt], BF)
                acc = acc + jnp.dot(vt, p.astype(BF), preferred_element_type=F32)
            q0 = pl.multiple_of(qi * 128, 128)
            ot_s[pl.ds(ro, DH), pl.ds(q0, 128)] = acc / l
            return c2

        lax.fori_loop(0, NLT, qblock, 0)
        return carry

    def stage_a(r0, n, h_w, hn_w, w0):
        o = ot_s[:, pl.ds(r0, n)].T.astype(BF)
        attn = jnp.dot(o, wo_s[...], preferred_element_type=F32)
        h = x_s[pl.ds(r0, n), :].astype(F32) + attn
        h_w[w0:w0 + n, :] = h
        hn_w[w0:w0 + n, :] = _layernorm(h).astype(BF)

    def first_a():
        stage_a(0, TM3 // 2, h_s, hn_s, 0)
        stage_a(TM3 // 2, TM3 // 2, h_s, hn_s, TM3 // 2)

    def fast_path():
        lax.fori_loop(0, H // 2, fast_body, 0)
        for b in range(NSTR):
            lt = (NQ - 1) * NSTR + b
            acc = sv_s[b, 0:DH, :]
            l8 = sv_s[b, DH:DH + 8, :]
            for (b_, n) in gdefer:
                if b_ == b:
                    p = vpu_scores(kb_b[n % NLT], qb_b[lt])
                    l8 = l8 + p[:8] + p[8:]
                    ar_s[srow(b, n, 7):srow(b, n, 7) + 16, :] = p.astype(BF)
            for n in defer[b]:
                row = srow(b, n, 0)
                pt = ar_s[row:row + 128, :]
                vt = pltpu.bitcast(vt_s[H - 1, n % NLT], BF)
                acc = acc + jnp.dot(vt, pt, preferred_element_type=F32)
            ot_s[(H - 1) * DH:H * DH, lt * 128:(lt + 1) * 128] = finish(acc, l8)
        first_a()

    def slow_path():
        lax.fori_loop(0, H, slow_head, 0)
        first_a()

    for c in c_rest:
        c.wait()
    lax.cond(safe, fast_path, slow_path)

    def ocp(i, r0, n):
        return pltpu.make_async_copy(out_s.at[pl.ds(r0, n)], out_hbm.at[pl.ds(r0, n)], osems.at[i])

    def ffn(i, prefetch):
        r0 = pl.multiple_of(i * TM3, TM3) if prefetch else i * TM3
        span = 2 * TM3 if prefetch else TM3
        hv = h_s.at[pl.ds(r0, span)]
        hnv = hn_s.at[pl.ds(r0, span)]
        u = jnp.dot(hnv[0:TM3, :], w1_s[...], preferred_element_type=F32)
        u = _gelu(u + b1_s[...].astype(F32).reshape(1, F)).astype(BF)
        if prefetch:
            stage_a(pl.multiple_of(r0 + TM3, TM3), TM3, hv, hnv, TM3)
        b2v = b2_s[...].astype(F32).reshape(1, D)
        nparts = 1 if prefetch else 2
        n = TM3 // nparts
        for t in range(nparts):
            y = jnp.dot(u[t * n:(t + 1) * n], w2_s[...], preferred_element_type=F32) + b2v
            out_s[pl.ds(r0 + t * n, n), :] = (hv[t * n:(t + 1) * n, :] + y).astype(out_s.dtype)
            ocp(i + t, r0 + t * n, n).start()

    def ffn_body(i, c):
        ffn(i, True)
        return c

    lax.fori_loop(0, n3 - 1, ffn_body, 0)
    ffn(n3 - 1, False)
    for i in range(n3 - 1):
        ocp(i, i * TM3, TM3).wait()
    for t in range(2):
        ocp(n3 - 1 + t, (n3 - 1) * TM3 + t * (TM3 // 2), TM3 // 2).wait()


@jax.jit
def pallas_sequential_preLN__softmax_full_mha__dense_activation_gelu__prompt_kernel(
    A_x: jax.Array,
    A_wqkv: jax.Array,
    A_wo: jax.Array,
    B_x: jax.Array,
    B_w1: jax.Array,
    B_b1: jax.Array,
    B_w2: jax.Array,
    B_b2: jax.Array,
):
    B, S, D = A_x.shape
    F = B_w1.shape[1]
    assert B == 1 and D // H == 16 and S % (128 * NSTR) == 0
    x = A_x.reshape(S, D)
    n1 = S // TM1
    nlt = S // 128
    dh = D // H
    arows = NSTR * NR * 128 + (H // 2) * nlt * 16 + nlt * D
    any_spec = pl.BlockSpec(memory_space=pl.ANY)
    out = pl.pallas_call(
        functools.partial(_kernel, S=S, D=D, F=F),
        out_shape=jax.ShapeDtypeStruct((S, D), A_x.dtype),
        in_specs=[any_spec] * 7,
        out_specs=any_spec,
        scratch_shapes=[
            pltpu.VMEM((S, D), BF),
            pltpu.VMEM((3, D, D), BF),
            pltpu.VMEM((D, D), BF),
            pltpu.VMEM((D, F), BF),
            pltpu.VMEM((F, D), BF),
            pltpu.VMEM((2 * D, D), BF),
            pltpu.VMEM((TM1, D), BF),
            pltpu.VMEM((D, 128), BF),
            pltpu.VMEM((128, D), BF),
            pltpu.VMEM((8, TM1), F32),
            pltpu.VMEM((H // 2, S // 2, 128), U32),
            pltpu.VMEM((H, nlt, 8, 128), U32),
            pltpu.VMEM((H, nlt, 8, 128), U32),
            pltpu.VMEM((nlt, dh, 16, 128), F32),
            pltpu.VMEM((nlt, dh, 16, 128), F32),
            pltpu.VMEM((nlt, dh, 8, 128), F32),
            pltpu.VMEM((nlt, dh, 8, 128), F32),
            pltpu.VMEM((arows, 128), BF),
            pltpu.VMEM((NSTR + 1, 32, 128), F32),
            pltpu.VMEM((D, S), F32),
            pltpu.VMEM((S, 128), F32),
            pltpu.VMEM((S, D), BF),
            pltpu.VMEM((S, D), F32),
            pltpu.VMEM((S, D), BF),
            pltpu.VMEM((F,), BF),
            pltpu.VMEM((D,), BF),
            pltpu.SemaphoreType.DMA((3 + n1 + 5,)),
            pltpu.SemaphoreType.DMA((S // TM3 + 1,)),
        ],
        compiler_params=pltpu.CompilerParams(vmem_limit_bytes=100 * 1024 * 1024),
    )(x, A_wqkv, A_wo, B_w1, B_b1, B_w2, B_b2)
    return out.reshape(B, S, D)
```

```python
import functools
import math

import jax
import jax.numpy as jnp
from jax import lax
import jax.experimental.pallas as pl
import jax.experimental.pallas.tpu as pltpu

BF = jnp.bfloat16
F32 = jnp.float32
U32 = jnp.uint32

H = 32
LN_EPS = 1e-5
LOG2E = 1.4426950408889634

TM1 = 512
TM3 = 256

NSTR = 4
LAGU = 14
DL = 170
VL = 144
PLD = 56
GD = 140
KS = 4
QS = 4
P0 = 200
P1 = 300
NR = 4

SAFE_B = 60.0
SAFE_V_HI = 2.0 ** 40
SAFE_V_LO = 2.0 ** -40


def _nt(a, b):
    return lax.dot_general(a, b, (((1,), (1,)), ((), ())), preferred_element_type=F32)


def _layernorm(x):
    m = jnp.mean(x, axis=-1, keepdims=True)
    xc = x - m
    v = jnp.mean(xc * xc, axis=-1, keepdims=True)
    return xc * lax.rsqrt(v + LN_EPS)


def _gelu(x):
    c = math.sqrt(2.0 / math.pi)
    return 0.5 * x * (1.0 + jnp.tanh(c * (x + 0.044715 * (x * x * x))))


def _check_events(events, nq, nlt):
    nt = nq * nlt
    assert nt % NR == 0
    ring = {}
    for blk in range(2):
        over = set()
        for e in events:
            b, kind = e[2], e[3]
            if kind == 'post':
                n = e[4][0] * nlt + e[4][1]
                assert ring.get((b, n % NR, e[4][2])) is None
                ring[(b, n % NR, e[4][2])] = (blk, n)
            elif kind == 'vpu':
                df, n = e[4:]
                if df:
                    assert ('kb', n % nlt) not in over and ('qb', (n // nlt) * NSTR + b) not in over
                assert ring.get((b, n % NR, 7)) is None
                ring[(b, n % NR, 7)] = (blk - df, n)
            elif kind == 'pvld':
                df, n = e[4:]
                for i in range(8):
                    got = ring.pop((b, n % NR, i), None)
                    assert blk - df < 0 or got == (blk - df, n)
            elif kind in ('kb', 'qb'):
                over.add((kind, e[4]))


def _attention_events(nq, nlt):
    nt = nq * nlt
    events = []
    defer = {}
    gdefer = []
    period = 0
    for b in range(NSTR):
        units = [(n // nlt, n % nlt, i) for n in range(nt) for i in range(7)]
        tot = len(units)
        lagu = LAGU + 2 * b
        pts = []
        for n in range(nt):
            pos = 7 * (n + 1) + lagu
            pts.append((pos - tot, 1, n) if pos >= tot else (pos, 0, n))
        pts.sort()
        defer[b] = [p[2] for p in pts if p[1]]
        cuts = sorted(set([0, tot] + [p[0] for p in pts] + [7 * nlt * (q + 1) for q in range(nq)]))
        tm = 0
        pi = 0
        tpv = {}
        for lo, hi in zip(cuts, cuts[1:] + [None]):
            while pi < len(pts) and pts[pi][0] == lo:
                _, df, n = pts[pi]
                events.append((tm - PLD, 1, b, 'pvld', df, n))
                events.append((tm, 2, b, 'pv', df, n))
                tpv[n] = (tm, df)
                tm += 16
                pi += 1
            if hi is None:
                break
            events.append((tm, 2, b, 'qk', tuple(units[lo:hi])))
            for r in range(lo, hi):
                events.append((tm + (r - lo) * 16 + DL, 0, b, 'post', units[r]))
            tm += (hi - lo) * 16
        period = tm
        for n in range(nt):
            t, df = tpv[n]
            tg = t + (period if df else 0) - VL
            if tg >= period + GD:
                events.append((tg - period, 0, b, 'vpu', 1, n))
                gdefer.append((b, n))
            else:
                events.append((tg, 0, b, 'vpu', 0, n))
        events.append((10 ** 9, 0, b, 'save'))
    pre = []
    for x in range(nlt):
        pre += [('kb', x, i) for i in range(KS)] + [('qb', x, i) for i in range(QS)]
    for n, e in enumerate(pre):
        events.append((P0 + (period - P0 - P1) * n // len(pre), 3, 0) + e)
    events.sort(key=lambda e: e[:3])
    _check_events(events, nq, nlt)
    return events, defer, gdefer


def _kernel(x_hbm, wqkv_hbm, wo_hbm, w1_hbm, b1_hbm, w2_hbm, b2_hbm, out_hbm,
            x_s, wqkv_s, wo_s, w1_s, w2_s, wqvt_s, xn0_s, q2_s, k2_s, v8_s,
            kr_s, qt_s, vt_s, kb_a, kb_b, qb_a, qb_b, ar_s, sv_s, ot_s, st_s, out_s, h_s, hn_s, b1_s, b2_s,
            sems, osems, *, S, D, F):
    DH = D // H
    NG = D // 128
    HPG = 128 // DH
    NLT = S // 128
    NQ = NLT // NSTR
    n1 = S // TM1
    n3 = S // TM3
    qscale = (DH ** -0.5) * LOG2E
    RING = NSTR * NR * 128
    KU0 = RING
    QU0 = KU0 + (H // 2) * NLT * 16

    def cp(src, dst, i):
        return pltpu.make_async_copy(src, dst, sems.at[i])

    def wcols(p):
        return cp(wqkv_hbm.at[:, pl.ds(p * D, D)], wqkv_s.at[p], p)

    c_wq, c_wk, c_wv = wcols(0), wcols(1), wcols(2)
    c_x = [cp(x_hbm.at[pl.ds(i * TM1, TM1)], x_s.at[pl.ds(i * TM1, TM1)], 3 + i) for i in range(n1)]
    rest = [(wo_hbm, wo_s), (w1_hbm, w1_s), (b1_hbm, b1_s), (w2_hbm, w2_s), (b2_hbm, b2_s)]
    c_rest = [cp(s_, d_, 3 + n1 + i) for i, (s_, d_) in enumerate(rest)]
    c_x[0].start()
    c_wq.start()
    c_wk.start()
    c_wv.start()
    for c in c_x[1:]:
        c.start()

    events, defer, gdefer = _attention_events(NQ, NLT)
    ar_s[0:RING, :] = jnp.zeros((RING, 128), BF)
    sv_s[...] = jnp.zeros(sv_s.shape, F32)
    sv_s[0:NSTR, DH:DH + 8, :] = jnp.ones((NSTR, 8, 128), F32)
    for u in sorted(set(n % NLT for _, n in gdefer)):
        kb_b[u] = jnp.zeros((DH, 16, 128), F32)
    for lt in sorted(set((n // NLT) * NSTR + b for b, n in gdefer)):
        qb_b[lt] = jnp.zeros((DH, 8, 128), F32)

    c_x[0].wait()
    xn0_s[...] = _layernorm(x_s[0:TM1, :].astype(F32)).astype(BF)

    def transpose_w(part, p):
        wqvt_s[part * D:(part + 1) * D, :] = wqkv_s[p].T

    c_wq.wait()
    transpose_w(0, 0)

    hi = lax.broadcasted_iota(jnp.int32, (H, D), 0)
    cj = lax.broadcasted_iota(jnp.int32, (H, D), 1)
    ind = jnp.where(cj // DH == hi, 1.0, 0.0).astype(BF)

    def kb_store(kb_w, u, kk, lo, ds=range(DH)):
        for d in ds:
            kb_w[u, d] = jnp.broadcast_to(kk[:, lo + d:lo + d + 1], (16, 128))

    def qb_store(qb_w, lt, qq, ds=range(DH)):
        for d in ds:
            qb_w[lt, d] = jnp.broadcast_to(qq[d:d + 1, :], (8, 128))

    nsub = TM1 // 128
    stats = {'q': None, 'k': None, 'v': None}

    def upd(name, val):
        stats[name] = val if stats[name] is None else jnp.maximum(stats[name], val)

    def norm_dots(q2, k2):
        upd('q', jnp.dot(ind, q2, preferred_element_type=F32))
        upd('k', _nt(ind, k2))

    def v_part(xn, r0, m0, m1):
        vb = _nt(wqvt_s[D + m0:D + m1, :], xn).astype(BF)
        vu = pltpu.bitcast(vb, U32)
        for t in range(nsub):
            vt_s[m0 // DH:m1 // DH, r0 // 128 + t] = (
                vu[:, t * 128:(t + 1) * 128].reshape((m1 - m0) // DH, 8, 128))
        upd('v', jnp.abs(vb.astype(F32)).reshape((m1 - m0) // 8, 8, TM1).max(axis=0))

    for i in range(n1):
        r0 = i * TM1
        xn = xn0_s[...] if i == 0 else _layernorm(x_s[r0:r0 + TM1, :].astype(F32)).astype(BF)
        qb = (_nt(wqvt_s[0:D, :], xn) * qscale).astype(BF)
        qu = pltpu.bitcast(qb, U32)
        qf = qb.astype(F32)
        for t in range(nsub):
            lt = r0 // 128 + t
            qt_s[:, lt] = qu[:, t * 128:(t + 1) * 128].reshape(H, 8, 128)
            for hh in range(H):
                row = QU0 + (hh * NLT + lt) * 16
                ar_s[row:row + 16, :] = qb[hh * DH:(hh + 1) * DH, t * 128:(t + 1) * 128]
            qb_store(qb_a, lt, qf[0:DH, t * 128:(t + 1) * 128])
        q2 = qf * qf
        q2 = functools.reduce(jnp.maximum, [q2[:, t * 128:(t + 1) * 128] for t in range(nsub)]).astype(BF)
        if i == 0:
            q2_s[...] = q2
            c_wk.wait()
            c_wv.wait()
            xn = xn0_s[...]
        kb = jnp.dot(xn, wqkv_s[1], preferred_element_type=F32).astype(BF)
        ku = pltpu.bitcast(kb, U32)
        kf = kb.astype(F32)
        for g in range(NG):
            kg = ku[:, g * 128:(g + 1) * 128]
            for jj in range(HPG // 2):
                hp2 = g * (HPG // 2) + jj
                kr = kg if jj == 0 else pltpu.roll(kg, 128 - jj * 2 * DH, 1)
                kr_s[hp2, r0 // 2:(r0 + TM1) // 2, :] = kr
                for t in range(nsub):
                    row = KU0 + (hp2 * NLT + r0 // 128 + t) * 16
                    ar_s[row:row + 16, :] = pltpu.bitcast(kr[t * 64 + 56:t * 64 + 64], BF)
        for t in range(nsub):
            kb_store(kb_a, r0 // 128 + t, kf[t * 128 + 112:(t + 1) * 128, 0:128], 0)
        k2 = kf * kf
        k2 = functools.reduce(jnp.maximum, [k2[t * 128:(t + 1) * 128] for t in range(nsub)]).astype(BF)
        if i == 0:
            transpose_w(1, 2)
        v_part(xn, r0, 0, D // 2)
        if i == 0:
            k2_s[...] = k2
            v8_s[...] = stats['v']
            for c in c_x[1:]:
                c.wait()
            for c in c_rest:
                c.start()
            xn = xn0_s[...]
            q2 = q2_s[...]
            k2 = k2_s[...]
            stats['v'] = v8_s[...]
        norm_dots(q2, k2)
        v_part(xn, r0, D // 2, D)

    qmax, kmax, vmax = stats['q'], stats['k'], stats['v']
    qh = jnp.max(qmax, axis=1, keepdims=True)
    kh = jnp.max(kmax, axis=1, keepdims=True)
    b2max = jnp.max(qh * kh) * 1.05
    vm = jnp.max(vmax)
    safe = jnp.logical_and(b2max <= SAFE_B * SAFE_B,
                           jnp.logical_and(vm <= SAFE_V_HI, vm >= SAFE_V_LO))


    def srow(b, n, i):
        return ((b * NR + n % NR) * 8 + i) * 16

    def finish(acc, l8):
        return acc / jnp.sum(l8, axis=0, keepdims=True)

    def vpu_scores(kb, qv):
        return jnp.exp2(jnp.sum(kb.reshape(DH, 2, 8, 128) * qv.reshape(DH, 1, 8, 128), axis=0))

    def fast_head(h, zero, odd, kb_r, qb_r, kb_w, qb_w):
        nz = 6
        zs = [zero * (i + 2) for i in range(nz)]
        cnt = [0]

        def nzero():
            cnt[0] += 1
            return zs[cnt[0] % nz]

        zrow = zero * 16
        h2 = lax.shift_right_logical(h, 1)
        ro = pl.multiple_of(h * DH, DH)
        hn = jnp.minimum(h + 1, H - 1)
        hn2 = lax.shift_right_logical(hn, 1)
        hp = jnp.maximum(h - 1, 0)
        rop = pl.multiple_of(hp * DH, DH)
        sval, accs, ls, pld = {}, {}, {}, {}

        ring = ar_s.at[pl.ds(pl.multiple_of(zrow, 16), RING)]
        ksrc = ar_s.at[pl.ds(pl.multiple_of(zrow + KU0 + hn2 * (NLT * 16), 16), NLT * 16)]
        qsrc = ar_s.at[pl.ds(pl.multiple_of(zrow + QU0 + hn * (NLT * 16), 16), NLT * 16)]
        for b in range(NSTR):
            ls[(1, (NQ - 1) * NSTR + b)] = sv_s[b, DH:DH + 8, :]

        pend = {}

        def take_l(key, extra=None):
            parts = [ls[key][None]] if key in ls else []
            parts += [p3[lo:hi] for p3, lo, hi in pend.pop(key, [])]
            if extra is not None:
                parts.append(extra)
            if len(parts) > 1 or key not in ls:
                ls[key] = jnp.sum(jnp.concatenate(parts, axis=0), axis=0)
            return ls[key]

        for ev in events:
            b, kind = ev[2], ev[3]
            if kind == 'qk':
                us = ev[4]
                lt = us[0][0] * NSTR + b
                runs = []
                for (_, j, i) in us:
                    r = j * 8 + i
                    if runs and runs[-1][1] == r:
                        runs[-1][1] = r + 1
                    else:
                        runs.append([r, r + 1])
                parts = [kr_s[h2, a * 8:c * 8, :] for a, c in runs]
                kc = parts[0] if len(parts) == 1 else jnp.concatenate(parts, axis=0)
                q = qt_s[h, lt]
                if odd:
                    q = jnp.concatenate([jnp.zeros_like(q), q], axis=0)
                kc = pltpu.bitcast(kc, BF)[:, :(2 * DH if odd else DH)]
                s = jnp.dot(kc, pltpu.bitcast(q, BF), preferred_element_type=F32)
                p = jnp.exp2(s)
                pb = p.astype(BF)
                p3 = p.reshape(2 * len(us), 8, 128)
                for n, u_ in enumerate(us):
                    sval[(b, u_)] = (p3, pb, n)
            elif kind == 'post':
                qi, j, i = ev[4]
                p3, pb, n = sval.pop((b, ev[4]))
                segs = pend.setdefault((0, qi * NSTR + b), [])
                if segs and segs[-1][0] is p3:
                    segs[-1] = (p3, segs[-1][1], 2 * n + 2)
                else:
                    segs.append((p3, 2 * n, 2 * n + 2))
                row = srow(b, qi * NLT + j, i)
                ar_s[row:row + 16, :] = pb[n * 16:(n + 1) * 16]
            elif kind == 'vpu':
                df, n = ev[4:]
                lt = (n // NLT) * NSTR + b
                if df:
                    p = vpu_scores(kb_w[n % NLT], qb_w[lt])
                else:
                    p = vpu_scores(kb_r[nzero() + n % NLT], qb_r[nzero() + lt])
                take_l((df, lt), p)
                row = srow(b, n, 7)
                ar_s[row:row + 16, :] = p.reshape(16, 128).astype(BF)
            elif kind == 'pvld':
                df, n = ev[4:]
                row = srow(b, n, 0)
                pld[(b, n)] = ring[row:row + 128, :]
            elif kind == 'pv':
                df, n = ev[4:]
                j = n % NLT
                lt = (n // NLT) * NSTR + b
                pt = pld.pop((b, n))
                vt = pltpu.bitcast(vt_s[hp if df else h, j], BF)
                key = (df, lt)
                if key not in accs:
                    accs[key] = sv_s[b if df else NSTR, 0:DH, :]
                accs[key] = accs[key] + jnp.dot(vt, pt, preferred_element_type=F32)
                if j == NLT - 1:
                    ot_s[pl.ds(rop if df else ro, DH), lt * 128:(lt + 1) * 128] = finish(accs[key], take_l(key))
            elif kind == 'save':
                lt = (NQ - 1) * NSTR + b
                sv_s[b, 0:DH, :] = accs[(0, lt)]
                sv_s[b, DH:DH + 8, :] = take_l((0, lt))
            elif kind == 'kb':
                row = ev[4] * 16
                ds = range(ev[5] * DH // KS, (ev[5] + 1) * DH // KS)
                kb_store(kb_w, ev[4], ksrc[row:row + 16, :].astype(F32), 0 if odd else DH, ds)
            elif kind == 'qb':
                row = ev[4] * 16
                ds = range(ev[5] * DH // QS, (ev[5] + 1) * DH // QS)
                qb_store(qb_w, ev[4], qsrc[row:row + 16, :].astype(F32), ds)

    def fast_body(h2, zero):
        @pl.when(zero == 0)
        def _():
            fast_head(2 * h2, zero, False, kb_a, qb_a, kb_b, qb_b)

        fast_head(2 * h2 + 1, zero, True, kb_b, qb_b, kb_a, qb_a)

        return zero * h2

    def slow_head(h, carry):
        ro = pl.multiple_of(h * DH, DH)

        def qblock(qi, c2):
            q = qt_s[h, qi]
            z = jnp.zeros_like(q)
            q = jnp.where((h & 1) == 1, jnp.concatenate([z, q], axis=0), jnp.concatenate([q, z], axis=0))
            q = pltpu.bitcast(q, BF)
            kc = pltpu.bitcast(kr_s[lax.shift_right_logical(h, 1)], BF)[:, :2 * DH]
            st_s[...] = jnp.dot(kc, q, preferred_element_type=F32)
            m = jnp.max(st_s[...], axis=0, keepdims=True)
            acc = jnp.zeros((DH, 128), F32)
            l = jnp.zeros((1, 128), F32)
            for kt in range(NLT):
                p = jnp.exp2(st_s[kt * 128:(kt + 1) * 128, :] - m)
                l = l + jnp.sum(p, axis=0, keepdims=True)
                vt = pltpu.bitcast(vt_s[h, kt], BF)
                acc = acc + jnp.dot(vt, p.astype(BF), preferred_element_type=F32)
            q0 = pl.multiple_of(qi * 128, 128)
            ot_s[pl.ds(ro, DH), pl.ds(q0, 128)] = acc / l
            return c2

        lax.fori_loop(0, NLT, qblock, 0)
        return carry

    def stage_a(r0, n, h_w, hn_w, w0):
        o = ot_s[:, pl.ds(r0, n)].T.astype(BF)
        attn = jnp.dot(o, wo_s[...], preferred_element_type=F32)
        h = x_s[pl.ds(r0, n), :].astype(F32) + attn
        h_w[w0:w0 + n, :] = h
        hn_w[w0:w0 + n, :] = _layernorm(h).astype(BF)

    def first_a():
        stage_a(0, TM3 // 2, h_s, hn_s, 0)
        stage_a(TM3 // 2, TM3 // 2, h_s, hn_s, TM3 // 2)

    def fast_path():
        lax.fori_loop(0, H // 2, fast_body, 0)
        for b in range(NSTR):
            lt = (NQ - 1) * NSTR + b
            acc = sv_s[b, 0:DH, :]
            l8 = sv_s[b, DH:DH + 8, :]
            for (b_, n) in gdefer:
                if b_ == b:
                    p = vpu_scores(kb_b[n % NLT], qb_b[lt])
                    l8 = l8 + p[0] + p[1]
                    ar_s[srow(b, n, 7):srow(b, n, 7) + 16, :] = p.reshape(16, 128).astype(BF)
            for n in defer[b]:
                row = srow(b, n, 0)
                pt = ar_s[row:row + 128, :]
                vt = pltpu.bitcast(vt_s[H - 1, n % NLT], BF)
                acc = acc + jnp.dot(vt, pt, preferred_element_type=F32)
            ot_s[(H - 1) * DH:H * DH, lt * 128:(lt + 1) * 128] = finish(acc, l8)
        first_a()

    def slow_path():
        lax.fori_loop(0, H, slow_head, 0)
        first_a()

    for c in c_rest:
        c.wait()
    lax.cond(safe, fast_path, slow_path)

    def ocp(i, r0, n):
        return pltpu.make_async_copy(out_s.at[pl.ds(r0, n)], out_hbm.at[pl.ds(r0, n)], osems.at[i])

    def ffn(i, prefetch):
        r0 = pl.multiple_of(i * TM3, TM3) if prefetch else i * TM3
        span = 2 * TM3 if prefetch else TM3
        hv = h_s.at[pl.ds(r0, span)]
        hnv = hn_s.at[pl.ds(r0, span)]
        u = jnp.dot(hnv[0:TM3, :], w1_s[...], preferred_element_type=F32)
        u = _gelu(u + b1_s[...].astype(F32).reshape(1, F)).astype(BF)
        if prefetch:
            stage_a(pl.multiple_of(r0 + TM3, TM3), TM3, hv, hnv, TM3)
        b2v = b2_s[...].astype(F32).reshape(1, D)
        nparts = 1 if prefetch else 2
        n = TM3 // nparts
        for t in range(nparts):
            y = jnp.dot(u[t * n:(t + 1) * n], w2_s[...], preferred_element_type=F32) + b2v
            out_s[pl.ds(r0 + t * n, n), :] = (hv[t * n:(t + 1) * n, :] + y).astype(out_s.dtype)
            ocp(i + t, r0 + t * n, n).start()

    def ffn_body(i, c):
        ffn(i, True)
        return c

    lax.fori_loop(0, n3 - 1, ffn_body, 0)
    ffn(n3 - 1, False)
    for i in range(n3 - 1):
        ocp(i, i * TM3, TM3).wait()
    for t in range(2):
        ocp(n3 - 1 + t, (n3 - 1) * TM3 + t * (TM3 // 2), TM3 // 2).wait()


@jax.jit
def pallas_sequential_preLN__softmax_full_mha__dense_activation_gelu__prompt_kernel(
    A_x: jax.Array,
    A_wqkv: jax.Array,
    A_wo: jax.Array,
    B_x: jax.Array,
    B_w1: jax.Array,
    B_b1: jax.Array,
    B_w2: jax.Array,
    B_b2: jax.Array,
):
    B, S, D = A_x.shape
    F = B_w1.shape[1]
    assert B == 1 and D // H == 16 and S % (128 * NSTR) == 0
    x = A_x.reshape(S, D)
    n1 = S // TM1
    nlt = S // 128
    dh = D // H
    arows = NSTR * NR * 128 + (H // 2) * nlt * 16 + nlt * D
    any_spec = pl.BlockSpec(memory_space=pl.ANY)
    out = pl.pallas_call(
        functools.partial(_kernel, S=S, D=D, F=F),
        out_shape=jax.ShapeDtypeStruct((S, D), A_x.dtype),
        in_specs=[any_spec] * 7,
        out_specs=any_spec,
        scratch_shapes=[
            pltpu.VMEM((S, D), BF),
            pltpu.VMEM((3, D, D), BF),
            pltpu.VMEM((D, D), BF),
            pltpu.VMEM((D, F), BF),
            pltpu.VMEM((F, D), BF),
            pltpu.VMEM((2 * D, D), BF),
            pltpu.VMEM((TM1, D), BF),
            pltpu.VMEM((D, 128), BF),
            pltpu.VMEM((128, D), BF),
            pltpu.VMEM((8, TM1), F32),
            pltpu.VMEM((H // 2, S // 2, 128), U32),
            pltpu.VMEM((H, nlt, 8, 128), U32),
            pltpu.VMEM((H, nlt, 8, 128), U32),
            pltpu.VMEM((nlt, dh, 16, 128), F32),
            pltpu.VMEM((nlt, dh, 16, 128), F32),
            pltpu.VMEM((nlt, dh, 8, 128), F32),
            pltpu.VMEM((nlt, dh, 8, 128), F32),
            pltpu.VMEM((arows, 128), BF),
            pltpu.VMEM((NSTR + 1, 32, 128), F32),
            pltpu.VMEM((D, S), F32),
            pltpu.VMEM((S, 128), F32),
            pltpu.VMEM((S, D), BF),
            pltpu.VMEM((S, D), F32),
            pltpu.VMEM((S, D), BF),
            pltpu.VMEM((F,), BF),
            pltpu.VMEM((D,), BF),
            pltpu.SemaphoreType.DMA((3 + n1 + 5,)),
            pltpu.SemaphoreType.DMA((S // TM3 + 1,)),
        ],
        compiler_params=pltpu.CompilerParams(vmem_limit_bytes=100 * 1024 * 1024),
    )(x, A_wqkv, A_wo, B_w1, B_b1, B_w2, B_b2)
    return out.reshape(B, S, D)
```

```python
import functools
import math

import jax
import jax.numpy as jnp
from jax import lax
import jax.experimental.pallas as pl
import jax.experimental.pallas.tpu as pltpu

BF = jnp.bfloat16
F32 = jnp.float32
U32 = jnp.uint32

H = 32
LN_EPS = 1e-5
LOG2E = 1.4426950408889634

TM1 = 512
TM3 = 256

NSTR = 4
LAGU = 14
DL = 170
VL = 144
PLD = 56
GD = 140
KS = 4
QS = 4
P0 = 200
P1 = 300
NR = 4

SAFE_B = 60.0
SAFE_V_HI = 2.0 ** 40
SAFE_V_LO = 2.0 ** -60


def _nt(a, b):
    return lax.dot_general(a, b, (((1,), (1,)), ((), ())), preferred_element_type=F32)


def _layernorm(x):
    m = jnp.mean(x, axis=-1, keepdims=True)
    xc = x - m
    v = jnp.mean(xc * xc, axis=-1, keepdims=True)
    return xc * lax.rsqrt(v + LN_EPS)


def _gelu(x):
    c = math.sqrt(2.0 / math.pi)
    return 0.5 * x * (1.0 + jnp.tanh(c * (x + 0.044715 * (x * x * x))))


def _check_events(events, nq, nlt):
    nt = nq * nlt
    assert nt % NR == 0
    ring = {}
    for blk in range(2):
        over = set()
        for e in events:
            b, kind = e[2], e[3]
            if kind == 'post':
                n = e[4][0] * nlt + e[4][1]
                assert ring.get((b, n % NR, e[4][2])) is None
                ring[(b, n % NR, e[4][2])] = (blk, n)
            elif kind == 'vpu':
                df, n = e[4:]
                if df:
                    assert ('kb', n % nlt) not in over and ('qb', (n // nlt) * NSTR + b) not in over
                assert ring.get((b, n % NR, 7)) is None
                ring[(b, n % NR, 7)] = (blk - df, n)
            elif kind == 'pvld':
                df, n = e[4:]
                for i in range(8):
                    got = ring.pop((b, n % NR, i), None)
                    assert blk - df < 0 or got == (blk - df, n)
            elif kind in ('kb', 'qb'):
                over.add((kind, e[4]))


def _attention_events(nq, nlt):
    nt = nq * nlt
    events = []
    defer = {}
    gdefer = []
    period = 0
    for b in range(NSTR):
        units = [(n // nlt, n % nlt, i) for n in range(nt) for i in range(7)]
        tot = len(units)
        lagu = LAGU + 2 * b
        pts = []
        for n in range(nt):
            pos = 7 * (n + 1) + lagu
            pts.append((pos - tot, 1, n) if pos >= tot else (pos, 0, n))
        pts.sort()
        defer[b] = [p[2] for p in pts if p[1]]
        cuts = sorted(set([0, tot] + [p[0] for p in pts] + [7 * nlt * (q + 1) for q in range(nq)]))
        tm = 0
        pi = 0
        tpv = {}
        for lo, hi in zip(cuts, cuts[1:] + [None]):
            while pi < len(pts) and pts[pi][0] == lo:
                _, df, n = pts[pi]
                events.append((tm - PLD, 1, b, 'pvld', df, n))
                events.append((tm, 2, b, 'pv', df, n))
                tpv[n] = (tm, df)
                tm += 16
                pi += 1
            if hi is None:
                break
            events.append((tm, 2, b, 'qk', tuple(units[lo:hi])))
            for r in range(lo, hi):
                events.append((tm + (r - lo) * 16 + DL, 0, b, 'post', units[r]))
            tm += (hi - lo) * 16
        period = tm
        for n in range(nt):
            t, df = tpv[n]
            tg = t + (period if df else 0) - VL
            if tg >= period + GD:
                events.append((tg - period, 0, b, 'vpu', 1, n))
                gdefer.append((b, n))
            else:
                events.append((tg, 0, b, 'vpu', 0, n))
        events.append((10 ** 9, 0, b, 'save'))
    pre = []
    for x in range(nlt):
        pre += [('kb', x, i) for i in range(KS)] + [('qb', x, i) for i in range(QS)]
    for n, e in enumerate(pre):
        events.append((P0 + (period - P0 - P1) * n // len(pre), 3, 0) + e)
    events.sort(key=lambda e: e[:3])
    _check_events(events, nq, nlt)
    return events, defer, gdefer


def _kernel(x_hbm, wqkv_hbm, wo_hbm, w1_hbm, b1_hbm, w2_hbm, b2_hbm, out_hbm,
            x_s, wqkv_s, wo_s, w1_s, w2_s, wqvt_s, xn0_s, q2_s, k2_s, v8_s,
            kr_s, qt_s, vt_s, kb_a, kb_b, qb_a, qb_b, ar_s, sv_s, ot_s, st_s, out_s, h_s, hn_s, b1_s, b2_s,
            sems, osems, *, S, D, F):
    DH = D // H
    NG = D // 128
    HPG = 128 // DH
    NLT = S // 128
    NQ = NLT // NSTR
    n1 = S // TM1
    n3 = S // TM3
    qscale = (DH ** -0.5) * LOG2E
    RING = NSTR * NR * 128
    KU0 = RING
    QU0 = KU0 + (H // 2) * NLT * 16

    def cp(src, dst, i):
        return pltpu.make_async_copy(src, dst, sems.at[i])

    def wcols(p):
        return cp(wqkv_hbm.at[:, pl.ds(p * D, D)], wqkv_s.at[p], p)

    c_wq, c_wk, c_wv = wcols(0), wcols(1), wcols(2)
    c_x = [cp(x_hbm.at[pl.ds(i * TM1, TM1)], x_s.at[pl.ds(i * TM1, TM1)], 3 + i) for i in range(n1)]
    rest = [(wo_hbm, wo_s), (w1_hbm, w1_s), (b1_hbm, b1_s), (w2_hbm, w2_s), (b2_hbm, b2_s)]
    c_rest = [cp(s_, d_, 3 + n1 + i) for i, (s_, d_) in enumerate(rest)]
    c_x[0].start()
    c_wq.start()
    c_wk.start()
    c_wv.start()
    for c in c_x[1:]:
        c.start()

    events, defer, gdefer = _attention_events(NQ, NLT)
    ar_s[0:RING, :] = jnp.zeros((RING, 128), BF)
    sv_s[...] = jnp.zeros(sv_s.shape, F32)
    sv_s[0:NSTR, DH:DH + 8, :] = jnp.ones((NSTR, 8, 128), F32)
    for u in sorted(set(n % NLT for _, n in gdefer)):
        kb_b[u] = jnp.zeros((DH, 16, 128), F32)
    for lt in sorted(set((n // NLT) * NSTR + b for b, n in gdefer)):
        qb_b[lt] = jnp.zeros((DH, 8, 128), F32)

    c_x[0].wait()
    xn0_s[...] = _layernorm(x_s[0:TM1, :].astype(F32)).astype(BF)

    def transpose_w(part, p):
        wqvt_s[part * D:(part + 1) * D, :] = wqkv_s[p].T

    c_wq.wait()
    transpose_w(0, 0)

    hi = lax.broadcasted_iota(jnp.int32, (H, D), 0)
    cj = lax.broadcasted_iota(jnp.int32, (H, D), 1)
    ind = jnp.where(cj // DH == hi, 1.0, 0.0).astype(BF)

    def kb_store(kb_w, u, kk, lo, ds=range(DH)):
        for d in ds:
            kb_w[u, d] = jnp.broadcast_to(kk[:, lo + d:lo + d + 1], (16, 128))

    def qb_store(qb_w, lt, qq, ds=range(DH)):
        for d in ds:
            qb_w[lt, d] = jnp.broadcast_to(qq[d:d + 1, :], (8, 128))

    nsub = TM1 // 128
    stats = {}

    def upd(name, val, op=jnp.maximum):
        stats[name] = op(stats[name], val) if name in stats else val

    def norm_dots(q2, k2):
        upd('q', jnp.dot(ind, q2, preferred_element_type=F32))
        upd('k', _nt(ind, k2))

    def v_part(xn, r0, m0, m1):
        vb = _nt(wqvt_s[D + m0:D + m1, :], xn).astype(BF)
        vu = pltpu.bitcast(vb, U32)
        for t in range(nsub):
            vt_s[m0 // DH:m1 // DH, r0 // 128 + t] = (
                vu[:, t * 128:(t + 1) * 128].reshape((m1 - m0) // DH, 8, 128))
        va = jnp.abs(vb.astype(F32)).reshape((m1 - m0) // 8, 8, TM1)
        upd('vhi', va.max(axis=0))
        upd('vlo', jnp.where(va == 0.0, 1.0, va).min(axis=0), jnp.minimum)

    for i in range(n1):
        r0 = i * TM1
        xn = xn0_s[...] if i == 0 else _layernorm(x_s[r0:r0 + TM1, :].astype(F32)).astype(BF)
        qb = (_nt(wqvt_s[0:D, :], xn) * qscale).astype(BF)
        qu = pltpu.bitcast(qb, U32)
        qf = qb.astype(F32)
        for t in range(nsub):
            lt = r0 // 128 + t
            qt_s[:, lt] = qu[:, t * 128:(t + 1) * 128].reshape(H, 8, 128)
            for hh in range(H):
                row = QU0 + (hh * NLT + lt) * 16
                ar_s[row:row + 16, :] = qb[hh * DH:(hh + 1) * DH, t * 128:(t + 1) * 128]
            qb_store(qb_a, lt, qf[0:DH, t * 128:(t + 1) * 128])
        q2 = qf * qf
        q2 = functools.reduce(jnp.maximum, [q2[:, t * 128:(t + 1) * 128] for t in range(nsub)]).astype(BF)
        if i == 0:
            q2_s[...] = q2
            c_wk.wait()
            c_wv.wait()
            xn = xn0_s[...]
        kb = jnp.dot(xn, wqkv_s[1], preferred_element_type=F32).astype(BF)
        ku = pltpu.bitcast(kb, U32)
        kf = kb.astype(F32)
        for g in range(NG):
            kg = ku[:, g * 128:(g + 1) * 128]
            for jj in range(HPG // 2):
                hp2 = g * (HPG // 2) + jj
                kr = kg if jj == 0 else pltpu.roll(kg, 128 - jj * 2 * DH, 1)
                kr_s[hp2, r0 // 2:(r0 + TM1) // 2, :] = kr
                for t in range(nsub):
                    row = KU0 + (hp2 * NLT + r0 // 128 + t) * 16
                    ar_s[row:row + 16, :] = pltpu.bitcast(kr[t * 64 + 56:t * 64 + 64], BF)
        for t in range(nsub):
            kb_store(kb_a, r0 // 128 + t, kf[t * 128 + 112:(t + 1) * 128, 0:128], 0)
        k2 = kf * kf
        k2 = functools.reduce(jnp.maximum, [k2[t * 128:(t + 1) * 128] for t in range(nsub)]).astype(BF)
        if i == 0:
            transpose_w(1, 2)
        v_part(xn, r0, 0, D // 2)
        if i == 0:
            k2_s[...] = k2
            v8_s[0] = stats['vhi']
            v8_s[1] = stats['vlo']
            for c in c_x[1:]:
                c.wait()
            for c in c_rest:
                c.start()
            xn = xn0_s[...]
            q2 = q2_s[...]
            k2 = k2_s[...]
            stats['vhi'] = v8_s[0]
            stats['vlo'] = v8_s[1]
        if i == n1 - 1:
            norm_dots(q2, k2)
        v_part(xn, r0, D // 2, D)
        if i < n1 - 1:
            norm_dots(q2, k2)

    qh = jnp.max(stats['q'], axis=1, keepdims=True)
    kh = jnp.max(stats['k'], axis=1, keepdims=True)
    b2max = jnp.max(qh * kh) * 1.05
    v_ok = jnp.logical_and(jnp.max(stats['vhi']) <= SAFE_V_HI, jnp.min(stats['vlo']) >= SAFE_V_LO)
    safe = jnp.logical_and(b2max <= SAFE_B * SAFE_B, v_ok)


    def srow(b, n, i):
        return ((b * NR + n % NR) * 8 + i) * 16

    def finish(acc, l8):
        return acc / jnp.sum(l8, axis=0, keepdims=True)

    def vpu_scores(kb, qv):
        return jnp.exp2(jnp.sum(kb.reshape(DH, 2, 8, 128) * qv.reshape(DH, 1, 8, 128), axis=0))

    def fast_head(h, zero, odd, kb_r, qb_r, kb_w, qb_w):
        nz = 6
        zs = [zero * (i + 2) for i in range(nz)]
        cnt = [0]

        def nzero():
            cnt[0] += 1
            return zs[cnt[0] % nz]

        zrow = zero * 16
        h2 = lax.shift_right_logical(h, 1)
        ro = pl.multiple_of(h * DH, DH)
        hn = jnp.minimum(h + 1, H - 1)
        hn2 = lax.shift_right_logical(hn, 1)
        hp = jnp.maximum(h - 1, 0)
        rop = pl.multiple_of(hp * DH, DH)
        sval, accs, ls, pld = {}, {}, {}, {}

        ring = ar_s.at[pl.ds(pl.multiple_of(zrow, 16), RING)]
        ksrc = ar_s.at[pl.ds(pl.multiple_of(zrow + KU0 + hn2 * (NLT * 16), 16), NLT * 16)]
        qsrc = ar_s.at[pl.ds(pl.multiple_of(zrow + QU0 + hn * (NLT * 16), 16), NLT * 16)]
        for b in range(NSTR):
            ls[(1, (NQ - 1) * NSTR + b)] = sv_s[b, DH:DH + 8, :]

        pend = {}

        def take_l(key, extra=None):
            parts = [ls[key][None]] if key in ls else []
            parts += [p3[lo:hi] for p3, lo, hi in pend.pop(key, [])]
            if extra is not None:
                parts.append(extra)
            if len(parts) > 1 or key not in ls:
                ls[key] = jnp.sum(jnp.concatenate(parts, axis=0), axis=0)
            return ls[key]

        for ev in events:
            b, kind = ev[2], ev[3]
            if kind == 'qk':
                us = ev[4]
                lt = us[0][0] * NSTR + b
                runs = []
                for (_, j, i) in us:
                    r = j * 8 + i
                    if runs and runs[-1][1] == r:
                        runs[-1][1] = r + 1
                    else:
                        runs.append([r, r + 1])
                parts = [kr_s[h2, a * 8:c * 8, :] for a, c in runs]
                kc = parts[0] if len(parts) == 1 else jnp.concatenate(parts, axis=0)
                q = qt_s[h, lt]
                if odd:
                    q = jnp.concatenate([jnp.zeros_like(q), q], axis=0)
                kc = pltpu.bitcast(kc, BF)[:, :(2 * DH if odd else DH)]
                s = jnp.dot(kc, pltpu.bitcast(q, BF), preferred_element_type=F32)
                p = jnp.exp2(s)
                pb = p.astype(BF)
                p3 = p.reshape(2 * len(us), 8, 128)
                for n, u_ in enumerate(us):
                    sval[(b, u_)] = (p3, pb, n)
            elif kind == 'post':
                qi, j, i = ev[4]
                p3, pb, n = sval.pop((b, ev[4]))
                segs = pend.setdefault((0, qi * NSTR + b), [])
                if segs and segs[-1][0] is p3:
                    segs[-1] = (p3, segs[-1][1], 2 * n + 2)
                else:
                    segs.append((p3, 2 * n, 2 * n + 2))
                row = srow(b, qi * NLT + j, i)
                ar_s[row:row + 16, :] = pb[n * 16:(n + 1) * 16]
            elif kind == 'vpu':
                df, n = ev[4:]
                lt = (n // NLT) * NSTR + b
                if df:
                    p = vpu_scores(kb_w[n % NLT], qb_w[lt])
                else:
                    p = vpu_scores(kb_r[nzero() + n % NLT], qb_r[nzero() + lt])
                take_l((df, lt), p)
                row = srow(b, n, 7)
                ar_s[row:row + 16, :] = p.reshape(16, 128).astype(BF)
            elif kind == 'pvld':
                df, n = ev[4:]
                row = srow(b, n, 0)
                pld[(b, n)] = ring[row:row + 128, :]
            elif kind == 'pv':
                df, n = ev[4:]
                j = n % NLT
                lt = (n // NLT) * NSTR + b
                pt = pld.pop((b, n))
                vt = pltpu.bitcast(vt_s[hp if df else h, j], BF)
                key = (df, lt)
                if key not in accs:
                    accs[key] = sv_s[b if df else NSTR, 0:DH, :]
                accs[key] = accs[key] + jnp.dot(vt, pt, preferred_element_type=F32)
                if j == NLT - 1:
                    ot_s[pl.ds(rop if df else ro, DH), lt * 128:(lt + 1) * 128] = finish(accs[key], take_l(key))
            elif kind == 'save':
                lt = (NQ - 1) * NSTR + b
                sv_s[b, 0:DH, :] = accs[(0, lt)]
                sv_s[b, DH:DH + 8, :] = take_l((0, lt))
            elif kind == 'kb':
                row = ev[4] * 16
                ds = range(ev[5] * DH // KS, (ev[5] + 1) * DH // KS)
                kb_store(kb_w, ev[4], ksrc[row:row + 16, :].astype(F32), 0 if odd else DH, ds)
            elif kind == 'qb':
                row = ev[4] * 16
                ds = range(ev[5] * DH // QS, (ev[5] + 1) * DH // QS)
                qb_store(qb_w, ev[4], qsrc[row:row + 16, :].astype(F32), ds)

    def fast_body(h2, zero):
        @pl.when(zero == 0)
        def _():
            fast_head(2 * h2, zero, False, kb_a, qb_a, kb_b, qb_b)

        fast_head(2 * h2 + 1, zero, True, kb_b, qb_b, kb_a, qb_a)

        return zero * h2

    def slow_head(h, carry):
        ro = pl.multiple_of(h * DH, DH)

        def qblock(qi, c2):
            q = qt_s[h, qi]
            z = jnp.zeros_like(q)
            q = jnp.where((h & 1) == 1, jnp.concatenate([z, q], axis=0), jnp.concatenate([q, z], axis=0))
            q = pltpu.bitcast(q, BF)
            kc = pltpu.bitcast(kr_s[lax.shift_right_logical(h, 1)], BF)[:, :2 * DH]
            st_s[...] = jnp.dot(kc, q, preferred_element_type=F32)
            m = jnp.max(st_s[...], axis=0, keepdims=True)
            acc = jnp.zeros((DH, 128), F32)
            l = jnp.zeros((1, 128), F32)
            for kt in range(NLT):
                p = jnp.exp2(st_s[kt * 128:(kt + 1) * 128, :] - m)
                l = l + jnp.sum(p, axis=0, keepdims=True)
                vt = pltpu.bitcast(vt_s[h, kt], BF)
                acc = acc + jnp.dot(vt, p.astype(BF), preferred_element_type=F32)
            q0 = pl.multiple_of(qi * 128, 128)
            ot_s[pl.ds(ro, DH), pl.ds(q0, 128)] = acc / l
            return c2

        lax.fori_loop(0, NLT, qblock, 0)
        return carry

    def stage_a(r0, n, h_w, hn_w, w0):
        o = ot_s[:, pl.ds(r0, n)].T.astype(BF)
        attn = jnp.dot(o, wo_s[...], preferred_element_type=F32)
        h = x_s[pl.ds(r0, n), :].astype(F32) + attn
        h_w[w0:w0 + n, :] = h
        hn_w[w0:w0 + n, :] = _layernorm(h).astype(BF)

    def first_a():
        stage_a(0, TM3 // 2, h_s, hn_s, 0)
        stage_a(TM3 // 2, TM3 // 2, h_s, hn_s, TM3 // 2)

    def fast_path():
        lax.fori_loop(0, H // 2, fast_body, 0)
        for b in range(NSTR):
            lt = (NQ - 1) * NSTR + b
            acc = sv_s[b, 0:DH, :]
            l8 = sv_s[b, DH:DH + 8, :]
            for (b_, n) in gdefer:
                if b_ == b:
                    p = vpu_scores(kb_b[n % NLT], qb_b[lt])
                    l8 = l8 + p[0] + p[1]
                    ar_s[srow(b, n, 7):srow(b, n, 7) + 16, :] = p.reshape(16, 128).astype(BF)
            for n in defer[b]:
                row = srow(b, n, 0)
                pt = ar_s[row:row + 128, :]
                vt = pltpu.bitcast(vt_s[H - 1, n % NLT], BF)
                acc = acc + jnp.dot(vt, pt, preferred_element_type=F32)
            ot_s[(H - 1) * DH:H * DH, lt * 128:(lt + 1) * 128] = finish(acc, l8)
        first_a()

    def slow_path():
        lax.fori_loop(0, H, slow_head, 0)
        first_a()

    for c in c_rest:
        c.wait()
    lax.cond(safe, fast_path, slow_path)

    def ocp(i, r0, n):
        return pltpu.make_async_copy(out_s.at[pl.ds(r0, n)], out_hbm.at[pl.ds(r0, n)], osems.at[i])

    def ffn(i, prefetch):
        r0 = pl.multiple_of(i * TM3, TM3) if prefetch else i * TM3
        span = 2 * TM3 if prefetch else TM3
        hv = h_s.at[pl.ds(r0, span)]
        hnv = hn_s.at[pl.ds(r0, span)]
        u = jnp.dot(hnv[0:TM3, :], w1_s[...], preferred_element_type=F32)
        u = _gelu(u + b1_s[...].astype(F32).reshape(1, F)).astype(BF)
        if prefetch:
            stage_a(pl.multiple_of(r0 + TM3, TM3), TM3, hv, hnv, TM3)
        b2v = b2_s[...].astype(F32).reshape(1, D)
        nparts = 1 if prefetch else 2
        n = TM3 // nparts
        for t in range(nparts):
            y = jnp.dot(u[t * n:(t + 1) * n], w2_s[...], preferred_element_type=F32) + b2v
            out_s[pl.ds(r0 + t * n, n), :] = (hv[t * n:(t + 1) * n, :] + y).astype(out_s.dtype)
            ocp(i + t, r0 + t * n, n).start()

    def ffn_body(i, c):
        ffn(i, True)
        return c

    lax.fori_loop(0, n3 - 1, ffn_body, 0)
    ffn(n3 - 1, False)
    for i in range(n3 - 1):
        ocp(i, i * TM3, TM3).wait()
    for t in range(2):
        ocp(n3 - 1 + t, (n3 - 1) * TM3 + t * (TM3 // 2), TM3 // 2).wait()


@jax.jit
def pallas_sequential_preLN__softmax_full_mha__dense_activation_gelu__prompt_kernel(
    A_x: jax.Array,
    A_wqkv: jax.Array,
    A_wo: jax.Array,
    B_x: jax.Array,
    B_w1: jax.Array,
    B_b1: jax.Array,
    B_w2: jax.Array,
    B_b2: jax.Array,
):
    B, S, D = A_x.shape
    F = B_w1.shape[1]
    assert B == 1 and D // H == 16 and S % (128 * NSTR) == 0
    x = A_x.reshape(S, D)
    n1 = S // TM1
    nlt = S // 128
    dh = D // H
    arows = NSTR * NR * 128 + (H // 2) * nlt * 16 + nlt * D
    any_spec = pl.BlockSpec(memory_space=pl.ANY)
    out = pl.pallas_call(
        functools.partial(_kernel, S=S, D=D, F=F),
        out_shape=jax.ShapeDtypeStruct((S, D), A_x.dtype),
        in_specs=[any_spec] * 7,
        out_specs=any_spec,
        scratch_shapes=[
            pltpu.VMEM((S, D), BF),
            pltpu.VMEM((3, D, D), BF),
            pltpu.VMEM((D, D), BF),
            pltpu.VMEM((D, F), BF),
            pltpu.VMEM((F, D), BF),
            pltpu.VMEM((2 * D, D), BF),
            pltpu.VMEM((TM1, D), BF),
            pltpu.VMEM((D, 128), BF),
            pltpu.VMEM((128, D), BF),
            pltpu.VMEM((2, 8, TM1), F32),
            pltpu.VMEM((H // 2, S // 2, 128), U32),
            pltpu.VMEM((H, nlt, 8, 128), U32),
            pltpu.VMEM((H, nlt, 8, 128), U32),
            pltpu.VMEM((nlt, dh, 16, 128), F32),
            pltpu.VMEM((nlt, dh, 16, 128), F32),
            pltpu.VMEM((nlt, dh, 8, 128), F32),
            pltpu.VMEM((nlt, dh, 8, 128), F32),
            pltpu.VMEM((arows, 128), BF),
            pltpu.VMEM((NSTR + 1, 32, 128), F32),
            pltpu.VMEM((D, S), F32),
            pltpu.VMEM((S, 128), F32),
            pltpu.VMEM((S, D), BF),
            pltpu.VMEM((S, D), F32),
            pltpu.VMEM((S, D), BF),
            pltpu.VMEM((F,), BF),
            pltpu.VMEM((D,), BF),
            pltpu.SemaphoreType.DMA((3 + n1 + 5,)),
            pltpu.SemaphoreType.DMA((S // TM3 + 1,)),
        ],
        compiler_params=pltpu.CompilerParams(vmem_limit_bytes=100 * 1024 * 1024),
    )(x, A_wqkv, A_wo, B_w1, B_b1, B_w2, B_b2)
    return out.reshape(B, S, D)
```

```python
import functools
import math

import jax
import jax.numpy as jnp
from jax import lax
import jax.experimental.pallas as pl
import jax.experimental.pallas.tpu as pltpu

BF = jnp.bfloat16
F32 = jnp.float32
U32 = jnp.uint32

H = 32
LN_EPS = 1e-5
LOG2E = 1.4426950408889634

TM1 = 512
TM3 = 256

NSTR = 4
LAGU = 9
DL = 150
KS = 8
QS = 4
P0 = 300
P1 = 300
X0 = 200
X1 = 5000
XPOS = 3

SAFE_B = 60.0
SAFE_V_HI = 2.0 ** 40
SAFE_V_LO = 2.0 ** -60


def _nt(a, b):
    return lax.dot_general(a, b, (((1,), (1,)), ((), ())), preferred_element_type=F32)


def _layernorm(x):
    m = jnp.mean(x, axis=-1, keepdims=True)
    xc = x - m
    v = jnp.mean(xc * xc, axis=-1, keepdims=True)
    return xc * lax.rsqrt(v + LN_EPS)


def _gelu(x):
    c = math.sqrt(2.0 / math.pi)
    return 0.5 * x * (1.0 + jnp.tanh(c * (x + 0.044715 * (x * x * x))))


def _attention_events(nq, nlt):
    nm = nq * nlt - 1
    events = []
    defer = {}
    period = 0
    for b in range(NSTR):
        o = (1 + 2 * b + 7 - LAGU) % 7
        last = [(nm - 1, i) for i in range(7)]
        units = last[:o] + [(n, i) for n in range(nm - 1) for i in range(7)] + last[o:]
        tot = len(units)
        pts = []
        for n in range(nm):
            pos = o + 7 * (n + 1) + LAGU
            pts.append((pos - tot, 1, n) if pos > tot else (pos, 0, n))
        pts.append((min(pts)[0] + XPOS, 1, nm))
        pts.sort()
        defer[b] = [p[2] for p in pts if p[1]]
        assert all(n // nlt == nq - 1 for n in defer[b])
        qcuts = [r for r in range(1, tot) if units[r][0] // nlt != units[r - 1][0] // nlt or r == o]
        cuts = sorted(set([0, tot] + [p[0] for p in pts] + qcuts))
        tm = 0
        pi = 0
        tfirst = {}
        for lo, hi in zip(cuts, cuts[1:] + [None]):
            while pi < len(pts) and pts[pi][0] == lo:
                events.append((tm, 2, b, 'pv', pts[pi][1], pts[pi][2]))
                tm += 16
                pi += 1
            if hi is None:
                break
            events.append((tm, 2, b, 'qk', tuple(units[lo:hi])))
            for r in range(lo, hi):
                t = tm + (r - lo) * 16 + DL
                events.append((t, 0, b, 'post', units[r]))
                if r >= o:
                    tfirst.setdefault(units[r][0], t)
            tm += (hi - lo) * 16
        period = tm
        for n in range(nm):
            events.append((tfirst[n] - 1, 0, b, 'vpu', n))
        events.append((10 ** 9, 0, b, 'save'))
    xs = [(b, i, c) for i in range(8) for c in range(2) for b in range(NSTR)]
    for n, (b, i, c) in enumerate(xs):
        events.append((X0 + max(period - X0 - X1, 0) * n // len(xs), 3, b, 'vpx', i, c))
    pre = []
    for x in range(nlt + 7):
        pre += [('kb', x, i) for i in range(KS)]
        if x < nlt:
            pre += [('qb', x, i) for i in range(QS)]
    for n, e in enumerate(pre):
        events.append((P0 + max(period - P0 - P1, 0) * n // len(pre), 3, 0) + e)
    events.sort(key=lambda e: e[:3])
    return events, defer


def _kernel(x_hbm, wqkv_hbm, wo_hbm, w1_hbm, b1_hbm, w2_hbm, b2_hbm, out_hbm,
            x_s, wqkv_s, wo_s, w1_s, w2_s, wqvt_s, xn0_s, q2_s, k2_s, v8_s,
            kr_s, qt_s, vt_s, kb_a, kb_b, qb_a, qb_b, ar_s, rg_s, sv_s, ot_s, st_s, out_s, h_s, hn_s, b1_s, b2_s,
            sems, osems, *, S, D, F):
    DH = D // H
    NG = D // 128
    HPG = 128 // DH
    NLT = S // 128
    NQ = NLT // NSTR
    n1 = S // TM1
    n3 = S // TM3
    qscale = (DH ** -0.5) * LOG2E
    NT = NQ * NLT
    NU = NLT + 8
    KU0 = 32
    QU0 = KU0 + (H // 2) * NU * 16
    PERM = (6, 5, 4, 3, 2, 1, 0, 7)

    def cp(src, dst, i):
        return pltpu.make_async_copy(src, dst, sems.at[i])

    def wcols(p):
        return cp(wqkv_hbm.at[:, pl.ds(p * D, D)], wqkv_s.at[p], p)

    c_wq, c_wk, c_wv = wcols(0), wcols(1), wcols(2)
    c_x = [cp(x_hbm.at[pl.ds(i * TM1, TM1)], x_s.at[pl.ds(i * TM1, TM1)], 3 + i) for i in range(n1)]
    rest = [(wo_hbm, wo_s), (w1_hbm, w1_s), (b1_hbm, b1_s), (w2_hbm, w2_s), (b2_hbm, b2_s)]
    c_rest = [cp(s_, d_, 3 + n1 + i) for i, (s_, d_) in enumerate(rest)]
    c_x[0].start()
    c_wq.start()
    c_wk.start()
    c_wv.start()
    for c in c_x[1:]:
        c.start()

    events, defer = _attention_events(NQ, NLT)
    assert max(len(v) for v in defer.values()) <= rg_s.shape[2]
    rg_s[1] = jnp.zeros(rg_s.shape[1:], BF)
    sv_s[...] = jnp.zeros(sv_s.shape, F32)
    sv_s[0:NSTR, DH:DH + 8, :] = jnp.ones((NSTR, 8, 128), F32)

    c_x[0].wait()
    xn0_s[...] = _layernorm(x_s[0:TM1, :].astype(F32)).astype(BF)

    def transpose_w(part, p):
        wqvt_s[part * D:(part + 1) * D, :] = wqkv_s[p].T

    c_wq.wait()
    transpose_w(0, 0)

    hi = lax.broadcasted_iota(jnp.int32, (H, D), 0)
    cj = lax.broadcasted_iota(jnp.int32, (H, D), 1)
    ind = jnp.where(cj // DH == hi, 1.0, 0.0).astype(BF)

    def kb_store(kb_w, u, kk, lo, ds=range(DH)):
        for d in ds:
            kb_w[u, d] = jnp.broadcast_to(kk[:, lo + d:lo + d + 1], (16, 128))

    def qb_store(qb_w, lt, qq, ds=range(DH)):
        for d in ds:
            qb_w[lt, d] = jnp.broadcast_to(qq[d:d + 1, :], (8, 128))

    nsub = TM1 // 128
    stats = {}

    def upd(name, val, op=jnp.maximum):
        stats[name] = op(stats[name], val) if name in stats else val

    def norm_dots(q2, k2):
        upd('q', jnp.dot(ind, q2, preferred_element_type=F32))
        upd('k', _nt(ind, k2))

    def v_part(xn, r0, m0, m1):
        xp = jnp.concatenate([xn[t * 128 + u * 16:t * 128 + (u + 1) * 16]
                              for t in range(nsub) for u in PERM], axis=0)
        vb = _nt(wqvt_s[D + m0:D + m1, :], xp).astype(BF)
        vu = pltpu.bitcast(vb, U32)
        for t in range(nsub):
            vt_s[m0 // DH:m1 // DH, r0 // 128 + t] = (
                vu[:, t * 128:(t + 1) * 128].reshape((m1 - m0) // DH, 8, 128))
        va = jnp.abs(vb.astype(F32)).reshape((m1 - m0) // 8, 8, TM1)
        upd('vhi', va.max(axis=0))
        upd('vlo', jnp.where(va == 0.0, 1.0, va).min(axis=0), jnp.minimum)

    for i in range(n1):
        r0 = i * TM1
        xn = xn0_s[...] if i == 0 else _layernorm(x_s[r0:r0 + TM1, :].astype(F32)).astype(BF)
        qb = (_nt(wqvt_s[0:D, :], xn) * qscale).astype(BF)
        qu = pltpu.bitcast(qb, U32)
        qf = qb.astype(F32)
        for t in range(nsub):
            lt = r0 // 128 + t
            qt_s[:, lt] = qu[:, t * 128:(t + 1) * 128].reshape(H, 8, 128)
            for hh in range(H):
                row = QU0 + (hh * NLT + lt) * 16
                ar_s[row:row + 16, :] = qf[hh * DH:(hh + 1) * DH, t * 128:(t + 1) * 128]
            qb_store(qb_a, lt, qf[0:DH, t * 128:(t + 1) * 128])
        q2 = qf * qf
        q2 = functools.reduce(jnp.maximum, [q2[:, t * 128:(t + 1) * 128] for t in range(nsub)]).astype(BF)
        if i == 0:
            q2_s[...] = q2
            c_wk.wait()
            c_wv.wait()
            xn = xn0_s[...]
        kb = jnp.dot(xn, wqkv_s[1], preferred_element_type=F32).astype(BF)
        ku = pltpu.bitcast(kb, U32)
        kf = kb.astype(F32)
        for g in range(NG):
            kg = ku[:, g * 128:(g + 1) * 128]
            for jj in range(HPG // 2):
                hp2 = g * (HPG // 2) + jj
                kr = kg if jj == 0 else pltpu.roll(kg, 128 - jj * 2 * DH, 1)
                kr_s[hp2, r0 // 2:(r0 + TM1) // 2, :] = kr
                for t in range(nsub):
                    row = KU0 + (hp2 * NU + r0 // 128 + t) * 16
                    ar_s[row:row + 16, :] = pltpu.bitcast(kr[t * 64 + 56:t * 64 + 64], BF).astype(F32)
                if i == 0:
                    row = KU0 + (hp2 * NU + NLT) * 16
                    ar_s[row:row + 112, :] = pltpu.bitcast(kr[0:56], BF).astype(F32)
        for t in range(nsub):
            kb_store(kb_a, r0 // 128 + t, kf[t * 128 + 112:(t + 1) * 128, 0:128], 0)
        if i == 1 or n1 == 1:
            for u in range(7):
                kb_store(kb_a, NLT + u, ar_s[KU0 + (NLT + u) * 16:KU0 + (NLT + u + 1) * 16, :], 0)
        k2 = kf * kf
        k2 = functools.reduce(jnp.maximum, [k2[t * 128:(t + 1) * 128] for t in range(nsub)]).astype(BF)
        if i == 0:
            transpose_w(1, 2)
        v_part(xn, r0, 0, D // 2)
        if i == 0:
            k2_s[...] = k2
            v8_s[0] = stats['vhi']
            v8_s[1] = stats['vlo']
            for c in c_x[1:]:
                c.wait()
            for c in c_rest:
                c.start()
            xn = xn0_s[...]
            q2 = q2_s[...]
            k2 = k2_s[...]
            stats['vhi'] = v8_s[0]
            stats['vlo'] = v8_s[1]
        if i == n1 - 1:
            norm_dots(q2, k2)
        v_part(xn, r0, D // 2, D)
        if i < n1 - 1:
            norm_dots(q2, k2)

    qh = jnp.max(stats['q'], axis=1, keepdims=True)
    kh = jnp.max(stats['k'], axis=1, keepdims=True)
    b2max = jnp.max(qh * kh) * 1.05
    v_ok = jnp.logical_and(jnp.max(stats['vhi']) <= SAFE_V_HI, jnp.min(stats['vlo']) >= SAFE_V_LO)
    safe = jnp.logical_and(b2max <= SAFE_B * SAFE_B, v_ok)


    def finish(acc, l8):
        return acc / jnp.sum(l8, axis=0, keepdims=True)

    def fast_head(h, zero, odd, kb_r, qb_r, kb_w, qb_w):
        par = 1 if odd else 0
        zs = [zero * (i + 2) for i in range(NSTR)]
        zrow = zero * 8
        h2 = lax.shift_right_logical(h, 1)
        ro = pl.multiple_of(h * DH, DH)
        hn = jnp.minimum(h + 1, H - 1)
        hn2 = lax.shift_right_logical(hn, 1)
        hp = jnp.maximum(h - 1, 0)
        rop = pl.multiple_of(hp * DH, DH)
        ksrc = ar_s.at[pl.ds(pl.multiple_of(zrow + KU0 + hn2 * (NU * 16), 8), NU * 16)]
        qsrc = ar_s.at[pl.ds(pl.multiple_of(zrow + QU0 + hn * (NLT * 16), 8), NLT * 16)]
        qcur = ar_s.at[pl.ds(pl.multiple_of(zrow + QU0 + h * (NLT * 16), 8), NLT * 16)]
        sval, accs, ls, pend, npv = {}, {}, {}, {}, {}
        fresh = []
        count = [0, 0]

        def take_l(key, extra=None):
            parts = [ls[key][None]] if key in ls else []
            parts += [p3[lo:hi] for p3, lo, hi in pend.pop(key, [])]
            if extra is not None:
                parts.append(extra)
            if len(parts) > 1 or key not in ls:
                ls[key] = jnp.sum(jnp.concatenate(parts, axis=0), axis=0)
            return ls[key]

        def release():
            if fresh:
                r = (count[0] % 4) * 8
                count[0] += 1
                p, lo = fresh[-1]
                ar_s[r:r + 8, :] = p[lo:lo + 8]

        def stage(b, n, i, lo, p):
            row = PERM.index(i) * 16 + lo
            rg_s[par, b, NT - 1 - n, row:row + p.shape[0], :] = p.astype(BF)

        for ev in events:
            b, kind = ev[2], ev[3]
            if kind == 'qk':
                us = ev[4]
                lt = (us[0][0] // NLT) * NSTR + b
                runs = []
                for (n, i) in us:
                    r = ((n + 1) % NLT) * 8 + i
                    if runs and runs[-1][1] == r:
                        runs[-1][1] = r + 1
                    else:
                        runs.append([r, r + 1])
                parts = [kr_s[h2, a * 8:c * 8, :] for a, c in runs]
                kc = parts[0] if len(parts) == 1 else jnp.concatenate(parts, axis=0)
                q = qt_s[h, lt]
                if odd:
                    q = jnp.concatenate([jnp.zeros_like(q), q], axis=0)
                kc = pltpu.bitcast(kc, BF)[:, :(2 * DH if odd else DH)]
                p = jnp.exp2(jnp.dot(kc, pltpu.bitcast(q, BF), preferred_element_type=F32))
                p3 = p.reshape(2 * len(us), 8, 128)
                for r, u_ in enumerate(us):
                    sval[(b, u_)] = (p, p3, r)
            elif kind == 'post':
                n, i = ev[4]
                p, p3, r = sval[(b, ev[4])]
                segs = pend.setdefault((n // NLT) * NSTR + b, [])
                if segs and segs[-1][0] is p3:
                    segs[-1] = (p3, segs[-1][1], 2 * r + 2)
                else:
                    segs.append((p3, 2 * r, 2 * r + 2))
                fresh.append((p, r * 16 + 8))
                if n in defer[b]:
                    stage(b, n, i, 0, p[r * 16:(r + 1) * 16])
            elif kind == 'vpu':
                n = ev[4]
                lt = (n // NLT) * NSTR + b
                kb = kb_r[zs[b] + (n + 1) % NLT].reshape(DH, 2, 8, 128)
                qv = qb_r[zs[n % NSTR] + lt].reshape(DH, 1, 8, 128)
                p3 = jnp.exp2(jnp.sum(kb * qv, axis=0))
                take_l(lt, p3)
                p = p3.reshape(16, 128)
                if n in defer[b]:
                    stage(b, n, 7, 0, p)
                else:
                    sval[(b, (n, 7))] = (p, p3, 0)
            elif kind == 'vpx':
                i, c = ev[4:]
                lt = (NQ - 1) * NSTR + b
                release()
                count[1] += 1
                q0 = jnp.broadcast_to(qcur[lt * 16:lt * 16 + 8, :][0:1], (8, 128))
                qv = jnp.concatenate([q0[None], qb_r[zs[count[1] % NSTR] + lt, 1:DH]], axis=0)
                kb = kb_r[zs[b] + (0 if i == 7 else NLT + i), :, c * 8:(c + 1) * 8, :]
                p = jnp.exp2(jnp.sum(kb * qv, axis=0))
                ls[('x', b)] = ls[('x', b)] + p if ('x', b) in ls else p
                stage(b, NT - 1, i, c * 8, p)
            elif kind == 'pv':
                df, n = ev[4:]
                lt = (n // NLT) * NSTR + b
                if df:
                    pt = rg_s[1 - par, b, NT - 1 - n]
                else:
                    rows = []
                    for i in PERM:
                        p, _, r = sval.pop((b, (n, i)))
                        rows.append(p if i == 7 else p[r * 16:(r + 1) * 16])
                    pt = jnp.concatenate(rows, axis=0).astype(BF)
                vt = pltpu.bitcast(vt_s[hp if df else h, (n + 1) % NLT], BF)
                key = (df, lt)
                if key not in accs:
                    accs[key] = sv_s[b if df else NSTR, 0:DH, :]
                accs[key] = accs[key] + jnp.dot(vt, pt, preferred_element_type=F32)
                npv[key] = npv.get(key, 0) + 1
                if npv[key] == (len(defer[b]) if df else NLT):
                    l8 = sv_s[b, DH:DH + 8, :] if df else take_l(lt)
                    ot_s[pl.ds(rop if df else ro, DH), lt * 128:(lt + 1) * 128] = finish(accs[key], l8)
            elif kind == 'save':
                lt = (NQ - 1) * NSTR + b
                sv_s[b, 0:DH, :] = accs[(0, lt)]
                sv_s[b, DH:DH + 8, :] = take_l(lt) + ls[('x', b)]
            elif kind == 'kb':
                release()
                ds = range(ev[5] * DH // KS, (ev[5] + 1) * DH // KS)
                kb_store(kb_w, ev[4], ksrc[ev[4] * 16:(ev[4] + 1) * 16, :], 0 if odd else DH, ds)
            elif kind == 'qb':
                release()
                ds = range(ev[5] * DH // QS, (ev[5] + 1) * DH // QS)
                qb_store(qb_w, ev[4], qsrc[ev[4] * 16:(ev[4] + 1) * 16, :], ds)

    def fast_body(h2, zero):
        @pl.when(zero == 0)
        def _():
            fast_head(2 * h2, zero, False, kb_a, qb_a, kb_b, qb_b)

        fast_head(2 * h2 + 1, zero, True, kb_b, qb_b, kb_a, qb_a)

        return zero * h2

    def slow_head(h, carry):
        ro = pl.multiple_of(h * DH, DH)

        def qblock(qi, c2):
            q = qt_s[h, qi]
            z = jnp.zeros_like(q)
            q = jnp.where((h & 1) == 1, jnp.concatenate([z, q], axis=0), jnp.concatenate([q, z], axis=0))
            q = pltpu.bitcast(q, BF)
            kc = pltpu.bitcast(kr_s[lax.shift_right_logical(h, 1)], BF)[:, :2 * DH]
            st_s[...] = jnp.dot(kc, q, preferred_element_type=F32)
            m = jnp.max(st_s[...], axis=0, keepdims=True)
            acc = jnp.zeros((DH, 128), F32)
            l = jnp.zeros((1, 128), F32)
            for kt in range(NLT):
                p = jnp.exp2(st_s[kt * 128:(kt + 1) * 128, :] - m)
                l = l + jnp.sum(p, axis=0, keepdims=True)
                vt = pltpu.bitcast(vt_s[h, kt], BF)
                pt = jnp.concatenate([p[u * 16:(u + 1) * 16] for u in PERM], axis=0).astype(BF)
                acc = acc + jnp.dot(vt, pt, preferred_element_type=F32)
            q0 = pl.multiple_of(qi * 128, 128)
            ot_s[pl.ds(ro, DH), pl.ds(q0, 128)] = acc / l
            return c2

        lax.fori_loop(0, NLT, qblock, 0)
        return carry

    def stage_a(r0, n, h_w, hn_w, w0):
        o = ot_s[:, pl.ds(r0, n)].T.astype(BF)
        attn = jnp.dot(o, wo_s[...], preferred_element_type=F32)
        h = x_s[pl.ds(r0, n), :].astype(F32) + attn
        h_w[w0:w0 + n, :] = h
        hn_w[w0:w0 + n, :] = _layernorm(h).astype(BF)

    def first_a():
        stage_a(0, TM3 // 2, h_s, hn_s, 0)
        stage_a(TM3 // 2, TM3 // 2, h_s, hn_s, TM3 // 2)

    def fast_path():
        lax.fori_loop(0, H // 2, fast_body, 0)
        for b in range(NSTR):
            lt = (NQ - 1) * NSTR + b
            acc = sv_s[b, 0:DH, :]
            for n in defer[b]:
                vt = pltpu.bitcast(vt_s[H - 1, (n + 1) % NLT], BF)
                acc = acc + jnp.dot(vt, rg_s[1, b, NT - 1 - n], preferred_element_type=F32)
            ot_s[(H - 1) * DH:H * DH, lt * 128:(lt + 1) * 128] = finish(acc, sv_s[b, DH:DH + 8, :])
        first_a()

    def slow_path():
        lax.fori_loop(0, H, slow_head, 0)
        first_a()

    for c in c_rest:
        c.wait()
    lax.cond(safe, fast_path, slow_path)

    def ocp(i, r0, n):
        return pltpu.make_async_copy(out_s.at[pl.ds(r0, n)], out_hbm.at[pl.ds(r0, n)], osems.at[i])

    def ffn(i, prefetch):
        r0 = pl.multiple_of(i * TM3, TM3) if prefetch else i * TM3
        span = 2 * TM3 if prefetch else TM3
        hv = h_s.at[pl.ds(r0, span)]
        hnv = hn_s.at[pl.ds(r0, span)]
        u = jnp.dot(hnv[0:TM3, :], w1_s[...], preferred_element_type=F32)
        u = _gelu(u + b1_s[...].astype(F32).reshape(1, F)).astype(BF)
        if prefetch:
            stage_a(pl.multiple_of(r0 + TM3, TM3), TM3, hv, hnv, TM3)
        b2v = b2_s[...].astype(F32).reshape(1, D)
        nparts = 1 if prefetch else 2
        n = TM3 // nparts
        for t in range(nparts):
            y = jnp.dot(u[t * n:(t + 1) * n], w2_s[...], preferred_element_type=F32) + b2v
            out_s[pl.ds(r0 + t * n, n), :] = (hv[t * n:(t + 1) * n, :] + y).astype(out_s.dtype)
            ocp(i + t, r0 + t * n, n).start()

    def ffn_body(i, c):
        ffn(i, True)
        return c

    lax.fori_loop(0, n3 - 1, ffn_body, 0)
    ffn(n3 - 1, False)
    for i in range(n3 - 1):
        ocp(i, i * TM3, TM3).wait()
    for t in range(2):
        ocp(n3 - 1 + t, (n3 - 1) * TM3 + t * (TM3 // 2), TM3 // 2).wait()


@jax.jit
def pallas_sequential_preLN__softmax_full_mha__dense_activation_gelu__prompt_kernel(
    A_x: jax.Array,
    A_wqkv: jax.Array,
    A_wo: jax.Array,
    B_x: jax.Array,
    B_w1: jax.Array,
    B_b1: jax.Array,
    B_w2: jax.Array,
    B_b2: jax.Array,
):
    B, S, D = A_x.shape
    F = B_w1.shape[1]
    assert B == 1 and D // H == 16 and S % (128 * NSTR) == 0
    x = A_x.reshape(S, D)
    n1 = S // TM1
    nlt = S // 128
    dh = D // H
    arows = 32 + (H // 2) * (nlt + 8) * 16 + nlt * D
    any_spec = pl.BlockSpec(memory_space=pl.ANY)
    out = pl.pallas_call(
        functools.partial(_kernel, S=S, D=D, F=F),
        out_shape=jax.ShapeDtypeStruct((S, D), A_x.dtype),
        in_specs=[any_spec] * 7,
        out_specs=any_spec,
        scratch_shapes=[
            pltpu.VMEM((S, D), BF),
            pltpu.VMEM((3, D, D), BF),
            pltpu.VMEM((D, D), BF),
            pltpu.VMEM((D, F), BF),
            pltpu.VMEM((F, D), BF),
            pltpu.VMEM((2 * D, D), BF),
            pltpu.VMEM((TM1, D), BF),
            pltpu.VMEM((D, 128), BF),
            pltpu.VMEM((128, D), BF),
            pltpu.VMEM((2, 8, TM1), F32),
            pltpu.VMEM((H // 2, S // 2, 128), U32),
            pltpu.VMEM((H, nlt, 8, 128), U32),
            pltpu.VMEM((H, nlt, 8, 128), U32),
            pltpu.VMEM((nlt + 7, dh, 16, 128), F32),
            pltpu.VMEM((nlt + 7, dh, 16, 128), F32),
            pltpu.VMEM((nlt, dh, 8, 128), F32),
            pltpu.VMEM((nlt, dh, 8, 128), F32),
            pltpu.VMEM((arows, 128), F32),
            pltpu.VMEM((2, NSTR, 4, 128, 128), BF),
            pltpu.VMEM((NSTR + 1, 32, 128), F32),
            pltpu.VMEM((D, S), F32),
            pltpu.VMEM((S, 128), F32),
            pltpu.VMEM((S, D), BF),
            pltpu.VMEM((S, D), F32),
            pltpu.VMEM((S, D), BF),
            pltpu.VMEM((F,), BF),
            pltpu.VMEM((D,), BF),
            pltpu.SemaphoreType.DMA((3 + n1 + 5,)),
            pltpu.SemaphoreType.DMA((S // TM3 + 1,)),
        ],
        compiler_params=pltpu.CompilerParams(vmem_limit_bytes=100 * 1024 * 1024),
    )(x, A_wqkv, A_wo, B_w1, B_b1, B_w2, B_b2)
    return out.reshape(B, S, D)
```

```python
import functools
import math

import jax
import jax.numpy as jnp
from jax import lax
import jax.experimental.pallas as pl
import jax.experimental.pallas.tpu as pltpu

BF = jnp.bfloat16
F32 = jnp.float32
U32 = jnp.uint32

H = 32
LN_EPS = 1e-5
LOG2E = 1.4426950408889634

TM1 = 512
TM3 = 256

NSTR = 4
LAGU = 9
DL = 150
KS = 8
QS = 4
P0 = 300
P1 = 300
X0 = 200
X1 = 5000
XPOS = 3

SAFE_B = 60.0
SAFE_V_HI = 2.0 ** 40
SAFE_V_LO = 2.0 ** -60


def _nt(a, b):
    return lax.dot_general(a, b, (((1,), (1,)), ((), ())), preferred_element_type=F32)


def _layernorm(x):
    m = jnp.mean(x, axis=-1, keepdims=True)
    xc = x - m
    v = jnp.mean(xc * xc, axis=-1, keepdims=True)
    return xc * lax.rsqrt(v + LN_EPS)


def _gelu(x):
    c = math.sqrt(2.0 / math.pi)
    return 0.5 * x * (1.0 + jnp.tanh(c * (x + 0.044715 * (x * x * x))))


def _attention_events(nq, nlt):
    nm = nq * nlt - 1
    events = []
    defer = {}
    period = 0
    for b in range(NSTR):
        o = (1 + 2 * b + 7 - LAGU) % 7
        last = [(nm - 1, i) for i in range(7)]
        units = last[:o] + [(n, i) for n in range(nm - 1) for i in range(7)] + last[o:]
        tot = len(units)
        pts = []
        for n in range(nm):
            pos = o + 7 * (n + 1) + LAGU
            pts.append((pos - tot, 1, n) if pos > tot else (pos, 0, n))
        pts.append((min(pts)[0] + XPOS, 1, nm))
        pts.sort()
        defer[b] = [p[2] for p in pts if p[1]]
        assert all(n // nlt == nq - 1 for n in defer[b])
        qcuts = [r for r in range(1, tot) if units[r][0] // nlt != units[r - 1][0] // nlt or r == o]
        cuts = sorted(set([0, tot] + [p[0] for p in pts] + qcuts))
        tm = 0
        pi = 0
        tfirst = {}
        for lo, hi in zip(cuts, cuts[1:] + [None]):
            while pi < len(pts) and pts[pi][0] == lo:
                events.append((tm, 2, b, 'pv', pts[pi][1], pts[pi][2]))
                tm += 16
                pi += 1
            if hi is None:
                break
            events.append((tm, 2, b, 'qk', tuple(units[lo:hi])))
            for r in range(lo, hi):
                t = tm + (r - lo) * 16 + DL
                events.append((t, 0, b, 'post', units[r]))
                if r >= o:
                    tfirst.setdefault(units[r][0], t)
            tm += (hi - lo) * 16
        period = tm
        for n in range(nm):
            events.append((tfirst[n] - 1, 0, b, 'vpu', n))
        events.append((10 ** 9, 0, b, 'save'))
    xs = [(b, i, c) for i in range(8) for c in range(2) for b in range(NSTR)]
    for n, (b, i, c) in enumerate(xs):
        events.append((X0 + max(period - X0 - X1, 0) * n // len(xs), 3, b, 'vpx', i, c))
    pre = []
    for x in range(nlt + 7):
        pre += [('kb', x, i) for i in range(KS)]
        if x < nlt:
            pre += [('qb', x, i) for i in range(QS)]
    for n, e in enumerate(pre):
        events.append((P0 + max(period - P0 - P1, 0) * n // len(pre), 3, 0) + e)
    events.sort(key=lambda e: e[:3])
    return events, defer


def _kernel(x_hbm, wqkv_hbm, wo_hbm, w1_hbm, b1_hbm, w2_hbm, b2_hbm, out_hbm,
            x_s, wqkv_s, wo_s, w1_s, w2_s, wqvt_s, xn0_s, q2_s, k2_s, v8_s,
            kr_s, qt_s, vt_s, kb_a, kb_b, qb_a, qb_b, ar_s, rg_s, sv_s, ot_s, st_s, out_s, h_s, hn_s, b1_s, b2_s,
            sems, osems, *, S, D, F):
    DH = D // H
    NG = D // 128
    HPG = 128 // DH
    NLT = S // 128
    NQ = NLT // NSTR
    n1 = S // TM1
    n3 = S // TM3
    qscale = (DH ** -0.5) * LOG2E
    NT = NQ * NLT
    NU = NLT + 8
    KU0 = 32
    QU0 = KU0 + (H // 2) * NU * 16
    PERM = (6, 5, 4, 3, 2, 1, 0, 7)

    def cp(src, dst, i):
        return pltpu.make_async_copy(src, dst, sems.at[i])

    def wcols(p):
        return cp(wqkv_hbm.at[:, pl.ds(p * D, D)], wqkv_s.at[p], p)

    c_wq, c_wk, c_wv = wcols(0), wcols(1), wcols(2)
    c_x = [cp(x_hbm.at[pl.ds(i * TM1, TM1)], x_s.at[pl.ds(i * TM1, TM1)], 3 + i) for i in range(n1)]
    rest = [(wo_hbm, wo_s), (w1_hbm, w1_s), (b1_hbm, b1_s), (w2_hbm, w2_s), (b2_hbm, b2_s)]
    c_rest = [cp(s_, d_, 3 + n1 + i) for i, (s_, d_) in enumerate(rest)]
    c_x[0].start()
    c_wq.start()
    c_wk.start()
    c_wv.start()
    for c in c_x[1:]:
        c.start()

    events, defer = _attention_events(NQ, NLT)
    assert max(len(v) for v in defer.values()) <= rg_s.shape[2]
    rg_s[1] = jnp.zeros(rg_s.shape[1:], BF)
    sv_s[...] = jnp.zeros(sv_s.shape, F32)
    sv_s[0:NSTR, DH:DH + 8, :] = jnp.ones((NSTR, 8, 128), F32)

    c_x[0].wait()
    xn0_s[...] = _layernorm(x_s[0:TM1, :].astype(F32)).astype(BF)

    def transpose_w(part, p):
        wqvt_s[part * D:(part + 1) * D, :] = wqkv_s[p].T

    c_wq.wait()
    transpose_w(0, 0)

    hi = lax.broadcasted_iota(jnp.int32, (H, D), 0)
    cj = lax.broadcasted_iota(jnp.int32, (H, D), 1)
    ind = jnp.where(cj // DH == hi, 1.0, 0.0).astype(BF)

    def kb_store(kb_w, u, kk, lo, ds=range(DH)):
        for d in ds:
            kb_w[u, d] = jnp.broadcast_to(kk[:, lo + d:lo + d + 1], (16, 128))

    def qb_store(qb_w, lt, qq, ds=range(DH)):
        for d in ds:
            qb_w[lt, d] = jnp.broadcast_to(qq[d:d + 1, :], (8, 128))

    nsub = TM1 // 128
    stats = {}

    def upd(name, val, op=jnp.maximum):
        stats[name] = op(stats[name], val) if name in stats else val

    def norm_dots(q2, k2):
        upd('q', jnp.dot(ind, q2, preferred_element_type=F32))
        upd('k', _nt(ind, k2))

    def permuted(x):
        return jnp.concatenate([x[t * 128 + u * 16:t * 128 + (u + 1) * 16, :]
                                for t in range(nsub) for u in PERM], axis=0).astype(BF)

    def v_part(xp, r0, m0, m1):
        vb = _nt(wqvt_s[D + m0:D + m1, :], xp).astype(BF)
        vu = pltpu.bitcast(vb, U32)
        for t in range(nsub):
            vt_s[m0 // DH:m1 // DH, r0 // 128 + t] = (
                vu[:, t * 128:(t + 1) * 128].reshape((m1 - m0) // DH, 8, 128))
        va = jnp.abs(vb.astype(F32)).reshape((m1 - m0) // 8, 8, TM1)
        upd('vhi', va.max(axis=0))
        upd('vlo', jnp.where(va == 0.0, 1.0, va).min(axis=0), jnp.minimum)

    for i in range(n1):
        r0 = i * TM1
        if i == 0:
            xn = xn0_s[...]
        else:
            xf = _layernorm(x_s[r0:r0 + TM1, :].astype(F32))
            xn = xf.astype(BF)
            xp = permuted(xf)
        qb = (_nt(wqvt_s[0:D, :], xn) * qscale).astype(BF)
        qu = pltpu.bitcast(qb, U32)
        qf = qb.astype(F32)
        for t in range(nsub):
            lt = r0 // 128 + t
            qt_s[:, lt] = qu[:, t * 128:(t + 1) * 128].reshape(H, 8, 128)
            for hh in range(H):
                row = QU0 + (hh * NLT + lt) * 16
                ar_s[row:row + 16, :] = qf[hh * DH:(hh + 1) * DH, t * 128:(t + 1) * 128]
            qb_store(qb_a, lt, qf[0:DH, t * 128:(t + 1) * 128])
        q2 = qf * qf
        q2 = functools.reduce(jnp.maximum, [q2[:, t * 128:(t + 1) * 128] for t in range(nsub)]).astype(BF)
        if i == 0:
            q2_s[...] = q2
            c_wk.wait()
            c_wv.wait()
            xn = xn0_s[...]
            xp = permuted(xn0_s)
        kb = jnp.dot(xn, wqkv_s[1], preferred_element_type=F32).astype(BF)
        ku = pltpu.bitcast(kb, U32)
        kf = kb.astype(F32)
        for g in range(NG):
            kg = ku[:, g * 128:(g + 1) * 128]
            for jj in range(HPG // 2):
                hp2 = g * (HPG // 2) + jj
                kr = kg if jj == 0 else pltpu.roll(kg, 128 - jj * 2 * DH, 1)
                kr_s[hp2, r0 // 2:(r0 + TM1) // 2, :] = kr
                for t in range(nsub):
                    row = KU0 + (hp2 * NU + r0 // 128 + t) * 16
                    ar_s[row:row + 16, :] = pltpu.bitcast(kr[t * 64 + 56:t * 64 + 64], BF).astype(F32)
                if i == 0:
                    row = KU0 + (hp2 * NU + NLT) * 16
                    ar_s[row:row + 112, :] = pltpu.bitcast(kr[0:56], BF).astype(F32)
        for t in range(nsub):
            kb_store(kb_a, r0 // 128 + t, kf[t * 128 + 112:(t + 1) * 128, 0:128], 0)
        if i == 0:
            for u in range(7):
                kb_store(kb_a, NLT + u, ar_s[KU0 + (NLT + u) * 16:KU0 + (NLT + u + 1) * 16, :], 0)
        k2 = kf * kf
        k2 = functools.reduce(jnp.maximum, [k2[t * 128:(t + 1) * 128] for t in range(nsub)]).astype(BF)
        if i == 0:
            transpose_w(1, 2)
        v_part(xp, r0, 0, D // 2)
        if i == 0:
            k2_s[...] = k2
            v8_s[0] = stats['vhi']
            v8_s[1] = stats['vlo']
            for c in c_x[1:]:
                c.wait()
            for c in c_rest:
                c.start()
            xp = permuted(xn0_s)
            q2 = q2_s[...]
            k2 = k2_s[...]
            stats['vhi'] = v8_s[0]
            stats['vlo'] = v8_s[1]
        if i == n1 - 1:
            norm_dots(q2, k2)
        v_part(xp, r0, D // 2, D)
        if i < n1 - 1:
            norm_dots(q2, k2)

    qh = jnp.max(stats['q'], axis=1, keepdims=True)
    kh = jnp.max(stats['k'], axis=1, keepdims=True)
    b2max = jnp.max(qh * kh) * 1.05
    v_ok = jnp.logical_and(jnp.max(stats['vhi']) <= SAFE_V_HI, jnp.min(stats['vlo']) >= SAFE_V_LO)
    safe = jnp.logical_and(b2max <= SAFE_B * SAFE_B, v_ok)


    def finish(acc, l8):
        return acc / jnp.sum(l8, axis=0, keepdims=True)

    def fast_head(h, zero, odd, kb_r, qb_r, kb_w, qb_w):
        par = 1 if odd else 0
        zs = [zero * (i + 2) for i in range(NSTR)]
        zrow = zero * 8
        h2 = lax.shift_right_logical(h, 1)
        ro = pl.multiple_of(h * DH, DH)
        hn = jnp.minimum(h + 1, H - 1)
        hn2 = lax.shift_right_logical(hn, 1)
        hp = jnp.maximum(h - 1, 0)
        rop = pl.multiple_of(hp * DH, DH)
        ksrc = ar_s.at[pl.ds(pl.multiple_of(zrow + KU0 + hn2 * (NU * 16), 8), NU * 16)]
        qsrc = ar_s.at[pl.ds(pl.multiple_of(zrow + QU0 + hn * (NLT * 16), 8), NLT * 16)]
        qcur = ar_s.at[pl.ds(pl.multiple_of(zrow + QU0 + h * (NLT * 16), 8), NLT * 16)]
        sval, accs, ls, pend, npv = {}, {}, {}, {}, {}
        fresh = []
        count = [0, 0]

        def take_l(key, extra=None):
            parts = [ls[key][None]] if key in ls else []
            parts += [p3[lo:hi] for p3, lo, hi in pend.pop(key, [])]
            if extra is not None:
                parts.append(extra)
            if len(parts) > 1 or key not in ls:
                ls[key] = jnp.sum(jnp.concatenate(parts, axis=0), axis=0)
            return ls[key]

        def release():
            if fresh:
                r = (count[0] % 4) * 8
                count[0] += 1
                p, lo = fresh[-1]
                ar_s[r:r + 8, :] = p[lo:lo + 8]

        def stage(b, n, i, lo, p):
            row = PERM.index(i) * 16 + lo
            rg_s[par, b, NT - 1 - n, row:row + p.shape[0], :] = p.astype(BF)

        for ev in events:
            b, kind = ev[2], ev[3]
            if kind == 'qk':
                us = ev[4]
                lt = (us[0][0] // NLT) * NSTR + b
                runs = []
                for (n, i) in us:
                    r = ((n + 1) % NLT) * 8 + i
                    if runs and runs[-1][1] == r:
                        runs[-1][1] = r + 1
                    else:
                        runs.append([r, r + 1])
                parts = [kr_s[h2, a * 8:c * 8, :] for a, c in runs]
                kc = parts[0] if len(parts) == 1 else jnp.concatenate(parts, axis=0)
                q = qt_s[h, lt]
                if odd:
                    q = jnp.concatenate([jnp.zeros_like(q), q], axis=0)
                kc = pltpu.bitcast(kc, BF)[:, :(2 * DH if odd else DH)]
                p = jnp.exp2(jnp.dot(kc, pltpu.bitcast(q, BF), preferred_element_type=F32))
                p3 = p.reshape(2 * len(us), 8, 128)
                for r, u_ in enumerate(us):
                    sval[(b, u_)] = (p, p3, r)
            elif kind == 'post':
                n, i = ev[4]
                p, p3, r = sval[(b, ev[4])]
                segs = pend.setdefault((n // NLT) * NSTR + b, [])
                if segs and segs[-1][0] is p3:
                    segs[-1] = (p3, segs[-1][1], 2 * r + 2)
                else:
                    segs.append((p3, 2 * r, 2 * r + 2))
                fresh.append((p, r * 16 + 8))
                if n in defer[b]:
                    stage(b, n, i, 0, p[r * 16:(r + 1) * 16])
            elif kind == 'vpu':
                n = ev[4]
                lt = (n // NLT) * NSTR + b
                kb = kb_r[zs[b] + (n + 1) % NLT].reshape(DH, 2, 8, 128)
                qv = qb_r[zs[n % NSTR] + lt].reshape(DH, 1, 8, 128)
                p3 = jnp.exp2(jnp.sum(kb * qv, axis=0))
                take_l(lt, p3)
                p = p3.reshape(16, 128)
                if n in defer[b]:
                    stage(b, n, 7, 0, p)
                else:
                    sval[(b, (n, 7))] = (p, p3, 0)
            elif kind == 'vpx':
                i, c = ev[4:]
                lt = (NQ - 1) * NSTR + b
                release()
                count[1] += 1
                q0 = jnp.broadcast_to(qcur[lt * 16:lt * 16 + 8, :][0:1], (8, 128))
                qv = jnp.concatenate([q0[None], qb_r[zs[count[1] % NSTR] + lt, 1:DH]], axis=0)
                kb = kb_r[zs[b] + (0 if i == 7 else NLT + i), :, c * 8:(c + 1) * 8, :]
                p = jnp.exp2(jnp.sum(kb * qv, axis=0))
                ls[('x', b)] = ls[('x', b)] + p if ('x', b) in ls else p
                stage(b, NT - 1, i, c * 8, p)
            elif kind == 'pv':
                df, n = ev[4:]
                lt = (n // NLT) * NSTR + b
                if df:
                    pt = rg_s[1 - par, b, NT - 1 - n]
                else:
                    rows = []
                    for i in PERM:
                        p, _, r = sval.pop((b, (n, i)))
                        rows.append(p if i == 7 else p[r * 16:(r + 1) * 16])
                    pt = jnp.concatenate(rows, axis=0).astype(BF)
                vt = pltpu.bitcast(vt_s[hp if df else h, (n + 1) % NLT], BF)
                key = (df, lt)
                if key not in accs:
                    accs[key] = sv_s[b if df else NSTR, 0:DH, :]
                accs[key] = accs[key] + jnp.dot(vt, pt, preferred_element_type=F32)
                npv[key] = npv.get(key, 0) + 1
                if npv[key] == (len(defer[b]) if df else NLT):
                    l8 = sv_s[b, DH:DH + 8, :] if df else take_l(lt)
                    ot_s[pl.ds(rop if df else ro, DH), lt * 128:(lt + 1) * 128] = finish(accs[key], l8)
            elif kind == 'save':
                lt = (NQ - 1) * NSTR + b
                sv_s[b, 0:DH, :] = accs[(0, lt)]
                sv_s[b, DH:DH + 8, :] = take_l(lt) + ls[('x', b)]
            elif kind == 'kb':
                release()
                ds = range(ev[5] * DH // KS, (ev[5] + 1) * DH // KS)
                kb_store(kb_w, ev[4], ksrc[ev[4] * 16:(ev[4] + 1) * 16, :], 0 if odd else DH, ds)
            elif kind == 'qb':
                release()
                ds = range(ev[5] * DH // QS, (ev[5] + 1) * DH // QS)
                qb_store(qb_w, ev[4], qsrc[ev[4] * 16:(ev[4] + 1) * 16, :], ds)

    def fast_body(h2, zero):
        @pl.when(zero == 0)
        def _():
            fast_head(2 * h2, zero, False, kb_a, qb_a, kb_b, qb_b)

        fast_head(2 * h2 + 1, zero, True, kb_b, qb_b, kb_a, qb_a)

        return zero * h2

    def slow_head(h, carry):
        ro = pl.multiple_of(h * DH, DH)

        def qblock(qi, c2):
            q = qt_s[h, qi]
            z = jnp.zeros_like(q)
            q = jnp.where((h & 1) == 1, jnp.concatenate([z, q], axis=0), jnp.concatenate([q, z], axis=0))
            q = pltpu.bitcast(q, BF)
            kc = pltpu.bitcast(kr_s[lax.shift_right_logical(h, 1)], BF)[:, :2 * DH]
            st_s[...] = jnp.dot(kc, q, preferred_element_type=F32)
            m = jnp.max(st_s[...], axis=0, keepdims=True)
            acc = jnp.zeros((DH, 128), F32)
            l = jnp.zeros((1, 128), F32)
            for kt in range(NLT):
                p = jnp.exp2(st_s[kt * 128:(kt + 1) * 128, :] - m)
                l = l + jnp.sum(p, axis=0, keepdims=True)
                vt = pltpu.bitcast(vt_s[h, kt], BF)
                pt = jnp.concatenate([p[u * 16:(u + 1) * 16] for u in PERM], axis=0).astype(BF)
                acc = acc + jnp.dot(vt, pt, preferred_element_type=F32)
            q0 = pl.multiple_of(qi * 128, 128)
            ot_s[pl.ds(ro, DH), pl.ds(q0, 128)] = acc / l
            return c2

        lax.fori_loop(0, NLT, qblock, 0)
        return carry

    def stage_a(r0, n, h_w, hn_w, w0):
        o = ot_s[:, pl.ds(r0, n)].T.astype(BF)
        attn = jnp.dot(o, wo_s[...], preferred_element_type=F32)
        h = x_s[pl.ds(r0, n), :].astype(F32) + attn
        h_w[w0:w0 + n, :] = h
        hn_w[w0:w0 + n, :] = _layernorm(h).astype(BF)

    def first_a():
        stage_a(0, TM3 // 2, h_s, hn_s, 0)
        stage_a(TM3 // 2, TM3 // 2, h_s, hn_s, TM3 // 2)

    def fast_path():
        lax.fori_loop(0, H // 2, fast_body, 0)
        for b in range(NSTR):
            lt = (NQ - 1) * NSTR + b
            acc = sv_s[b, 0:DH, :]
            for n in defer[b]:
                vt = pltpu.bitcast(vt_s[H - 1, (n + 1) % NLT], BF)
                acc = acc + jnp.dot(vt, rg_s[1, b, NT - 1 - n], preferred_element_type=F32)
            ot_s[(H - 1) * DH:H * DH, lt * 128:(lt + 1) * 128] = finish(acc, sv_s[b, DH:DH + 8, :])
        first_a()

    def slow_path():
        lax.fori_loop(0, H, slow_head, 0)
        first_a()

    for c in c_rest:
        c.wait()
    lax.cond(safe, fast_path, slow_path)

    def ocp(i, r0, n):
        return pltpu.make_async_copy(out_s.at[pl.ds(r0, n)], out_hbm.at[pl.ds(r0, n)], osems.at[i])

    def ffn(i, prefetch):
        r0 = pl.multiple_of(i * TM3, TM3) if prefetch else i * TM3
        span = 2 * TM3 if prefetch else TM3
        hv = h_s.at[pl.ds(r0, span)]
        hnv = hn_s.at[pl.ds(r0, span)]
        u = jnp.dot(hnv[0:TM3, :], w1_s[...], preferred_element_type=F32)
        u = _gelu(u + b1_s[...].astype(F32).reshape(1, F)).astype(BF)
        if prefetch:
            stage_a(pl.multiple_of(r0 + TM3, TM3), TM3, hv, hnv, TM3)
        b2v = b2_s[...].astype(F32).reshape(1, D)
        nparts = 1 if prefetch else 2
        n = TM3 // nparts
        for t in range(nparts):
            y = jnp.dot(u[t * n:(t + 1) * n], w2_s[...], preferred_element_type=F32) + b2v
            out_s[pl.ds(r0 + t * n, n), :] = (hv[t * n:(t + 1) * n, :] + y).astype(out_s.dtype)
            ocp(i + t, r0 + t * n, n).start()

    def ffn_body(i, c):
        ffn(i, True)
        return c

    lax.fori_loop(0, n3 - 1, ffn_body, 0)
    ffn(n3 - 1, False)
    for i in range(n3 - 1):
        ocp(i, i * TM3, TM3).wait()
    for t in range(2):
        ocp(n3 - 1 + t, (n3 - 1) * TM3 + t * (TM3 // 2), TM3 // 2).wait()


@jax.jit
def pallas_sequential_preLN__softmax_full_mha__dense_activation_gelu__prompt_kernel(
    A_x: jax.Array,
    A_wqkv: jax.Array,
    A_wo: jax.Array,
    B_x: jax.Array,
    B_w1: jax.Array,
    B_b1: jax.Array,
    B_w2: jax.Array,
    B_b2: jax.Array,
):
    B, S, D = A_x.shape
    F = B_w1.shape[1]
    assert B == 1 and D // H == 16 and S % (128 * NSTR) == 0
    x = A_x.reshape(S, D)
    n1 = S // TM1
    nlt = S // 128
    dh = D // H
    arows = 32 + (H // 2) * (nlt + 8) * 16 + nlt * D
    any_spec = pl.BlockSpec(memory_space=pl.ANY)
    out = pl.pallas_call(
        functools.partial(_kernel, S=S, D=D, F=F),
        out_shape=jax.ShapeDtypeStruct((S, D), A_x.dtype),
        in_specs=[any_spec] * 7,
        out_specs=any_spec,
        scratch_shapes=[
            pltpu.VMEM((S, D), BF),
            pltpu.VMEM((3, D, D), BF),
            pltpu.VMEM((D, D), BF),
            pltpu.VMEM((D, F), BF),
            pltpu.VMEM((F, D), BF),
            pltpu.VMEM((2 * D, D), BF),
            pltpu.VMEM((TM1, D), BF),
            pltpu.VMEM((D, 128), BF),
            pltpu.VMEM((128, D), BF),
            pltpu.VMEM((2, 8, TM1), F32),
            pltpu.VMEM((H // 2, S // 2, 128), U32),
            pltpu.VMEM((H, nlt, 8, 128), U32),
            pltpu.VMEM((H, nlt, 8, 128), U32),
            pltpu.VMEM((nlt + 7, dh, 16, 128), F32),
            pltpu.VMEM((nlt + 7, dh, 16, 128), F32),
            pltpu.VMEM((nlt, dh, 8, 128), F32),
            pltpu.VMEM((nlt, dh, 8, 128), F32),
            pltpu.VMEM((arows, 128), F32),
            pltpu.VMEM((2, NSTR, 4, 128, 128), BF),
            pltpu.VMEM((NSTR + 1, 32, 128), F32),
            pltpu.VMEM((D, S), F32),
            pltpu.VMEM((S, 128), F32),
            pltpu.VMEM((S, D), BF),
            pltpu.VMEM((S, D), F32),
            pltpu.VMEM((S, D), BF),
            pltpu.VMEM((F,), BF),
            pltpu.VMEM((D,), BF),
            pltpu.SemaphoreType.DMA((3 + n1 + 5,)),
            pltpu.SemaphoreType.DMA((S // TM3 + 1,)),
        ],
        compiler_params=pltpu.CompilerParams(vmem_limit_bytes=100 * 1024 * 1024),
    )(x, A_wqkv, A_wo, B_w1, B_b1, B_w2, B_b2)
    return out.reshape(B, S, D)
```
